```python
import jax
import jax.numpy as jnp

def _softmax(x, axis=-1):
    return jax.nn.softmax(x, axis=axis)

def _gelu(x):
    return jax.nn.gelu(x, approximate=True)

def _silu(x):
    return jax.nn.silu(x)

def _sigmoid(x):
    return jax.nn.sigmoid(x)

def _layernorm(x, axis=-1, eps=1e-05):
    m = jnp.mean(x, axis=axis, keepdims=True)
    v = jnp.var(x, axis=axis, keepdims=True)
    return (x - m) / jnp.sqrt(v + eps)

def _scatter_add(tgt, idx, src, axis=0):
    return tgt.at[idx].add(src)

def _segment_sum(src, seg, n):
    return jax.ops.segment_sum(src, seg, n)

class _Rng:

    def __init__(self, key):
        self._k = key

    def _next(self):
        self._k, sub = jax.random.split(self._k)
        return sub

    def normal(self, shape):
        return jax.random.normal(self._next(), shape, dtype=jnp.bfloat16)

    def randint(self, lo, hi, shape):
        return jax.random.randint(self._next(), shape, lo, hi, dtype=jnp.int32)

    def uniform(self, shape, lo=0.0, hi=1.0):
        return jax.random.uniform(self._next(), shape, jnp.bfloat16, lo, hi)

    def permutation(self, n):
        return jax.random.permutation(self._next(), n)
kernel_name = 'sequential_preLN__memory_aug_recurrent_mem_tr__mixer_s_mlp__prompt'

def setup_inputs():
    _rng = _Rng(jax.random.key(int.from_bytes(__import__("os").urandom(4), "little")))
    _w = lambda a: (lambda t: t.astype(jnp.bfloat16) if jnp.issubdtype(t.dtype, jnp.floating) else t)(jnp.asarray(a))

    def _A_setup():
        B, S, Dm = (1, 2048, 1024)
        H, Dh = (32, 128)
        M, seg = (8, 32)
        seg = min(seg, S)
        S = S // seg * seg
        return {'x': _w((lambda *s: _rng.normal(s) * 0.05)(B, S, Dm)), 'mem0': _w((lambda *s: _rng.normal(s) * 0.05)(B, M, Dm)), 'Wq': _w((lambda *s: _rng.normal(s) * 0.05)(Dm, H, Dh) * Dm ** (-0.5)), 'Wk': _w((lambda *s: _rng.normal(s) * 0.05)(Dm, H, Dh) * Dm ** (-0.5)), 'Wv': _w((lambda *s: _rng.normal(s) * 0.05)(Dm, H, Dh) * Dm ** (-0.5)), 'Wo': _w((lambda *s: _rng.normal(s) * 0.05)(H, Dh, Dm) * (H * Dh) ** (-0.5)), 'seg_len': seg}
    _A_in = _A_setup()

    def _B_setup():
        B, S, D, F = (1, 2048, 1024, 3584)
        return {'x': _w((lambda *s: _rng.normal(s) * 0.05)(B, S, D)), 'w1': _w((lambda *s: _rng.normal(s) * 0.05)(D, D) * D ** (-0.5)), 'w2': _w((lambda *s: _rng.normal(s) * 0.05)(D, D) * D ** (-0.5)), 'w3': _w((lambda *s: _rng.normal(s) * 0.05)(D, F) * D ** (-0.5)), 'w4': _w((lambda *s: _rng.normal(s) * 0.05)(F, D) * F ** (-0.5))}
    _B_in = _B_setup()
    return {'A_x': _A_in['x'], 'A_mem0': _A_in['mem0'], 'A_Wq': _A_in['Wq'], 'A_Wk': _A_in['Wk'], 'A_Wv': _A_in['Wv'], 'A_Wo': _A_in['Wo'], 'A_seg_len': _A_in['seg_len'], 'B_x': _B_in['x'], 'B_w1': _B_in['w1'], 'B_w2': _B_in['w2'], 'B_w3': _B_in['w3'], 'B_w4': _B_in['w4']}

def reference(A_x, A_mem0, A_Wq, A_Wk, A_Wv, A_Wo, A_seg_len, B_x, B_w1, B_w2, B_w3, B_w4):

    def _A_ref(x, mem0, Wq, Wk, Wv, Wo, seg_len):
        B, S, Dm = x.shape
        H, Dh = (Wq.shape[1], Wq.shape[2])
        M = mem0.shape[1]
        scale = Dh ** (-0.5)
        n_seg = S // seg_len
        L = M + seg_len
        idx = jnp.arange(L)
        mask = (idx[:, None] < M) | (idx[:, None] >= idx[None, :])
        mem = mem0
        outs = []
        for s in range(n_seg):
            xs = x[:, s * seg_len:(s + 1) * seg_len, :].copy()
            h = jnp.concatenate([mem, xs], axis=1)
            q = jnp.einsum('btd,dhe->bhte', h, Wq)
            k = jnp.einsum('btd,dhe->bhte', h, Wk)
            v = jnp.einsum('btd,dhe->bhte', h, Wv)
            scores = jnp.einsum('bhqe,bhke->bhqk', q, k) * scale
            scores = jnp.where(mask[None, None], scores, -1000000000.0)
            p = _softmax(scores, axis=-1)
            o = jnp.einsum('bhqk,bhke->bhqe', p, v)
            o = jnp.einsum('bhte,hed->btd', o, Wo)
            mem = o[:, :M, :].copy()
            outs.append(o[:, M:, :])
        return jnp.concatenate(outs, axis=1)

    def _B_ref(x, w1, w2, w3, w4):
        B, S, D = x.shape
        h = _gelu(_layernorm(x, axis=-1) @ w1)
        c = D // 4
        g0 = jnp.pad(h[:, :, 0 * c:1 * c], ((0, 0), (1, 0), (0, 0)))[:, :S, :]
        g1 = jnp.pad(h[:, :, 1 * c:2 * c], ((0, 0), (0, 1), (0, 0)))[:, 1:, :]
        g2 = jnp.pad(h[:, :, 2 * c:3 * c], ((0, 0), (2, 0), (0, 0)))[:, :S, :]
        g3 = jnp.pad(h[:, :, 3 * c:], ((0, 0), (0, 2), (0, 0)))[:, 2:, :]
        hs = jnp.concatenate([g0, g1, g2, g3], axis=-1) @ w2
        x1 = x + hs
        h2 = _gelu(_layernorm(x1, axis=-1) @ w3) @ w4
        return x1 + h2
    x = A_x
    h = x + _A_ref(_layernorm(x, axis=-1), A_mem0, A_Wq, A_Wk, A_Wv, A_Wo, A_seg_len)
    h2 = h + _B_ref(_layernorm(h, axis=-1), B_w1, B_w2, B_w3, B_w4)
    return h2
```

```python
import functools

import jax
import jax.numpy as jnp
from jax import lax
import jax.experimental.pallas as pl
import jax.experimental.pallas.tpu as pltpu

S = 2048
D = 1024
H = 32
DH = 128
MEM = 8
SEG = 32
F = 3584
NSEG = S // SEG
L = MEM + SEG
TOK = 24
P0 = S - TOK * NSEG
RING = 576
XP = (S - P0) // 12
C4 = D // 4
HALO = 8
RB = 256
FC = 512
EPS = 1e-5
NEG = -1000000000.0

LAG_QK, LAG_PV, LAG_WO = 2, 4, 6
FILL_AT = 18
EARLY = 14
UNROLL = 2

bf16 = jnp.bfloat16
f32 = jnp.float32
u32 = jnp.uint32

SEM_X0, SEM_X, SEM_WO, SEM_W1, SEM_W2, SEM_W3, SEM_W4, SEM_OUT, SEM_W = (
    0, 1, 5, 9, 13, 14, 15, 16, 32)
NSEM = SEM_W + 12


def _mult(i, n):
    return i if isinstance(i, int) else pl.multiple_of(i, n)


def _ln(x):
    m = jnp.mean(x, axis=-1, keepdims=True)
    d = x - m
    v = jnp.mean(d * d, axis=-1, keepdims=True)
    return d * lax.rsqrt(v + EPS)


def _gelu(x):
    return jax.nn.gelu(x, approximate=True)


def _pack(x):
    return pltpu.bitcast(x.astype(bf16), u32)


def _unpack(x):
    return pltpu.bitcast(x, bf16)


def _pack2(even, odd):
    return pltpu.pack_elementwise([even, odd], packed_dtype=bf16)


def _half(w, i):
    return pltpu.unpack_elementwise(w, index=i, packed_dtype=bf16, unpacked_dtype=f32)


def _dot(a, b):
    return jnp.dot(a, b, preferred_element_type=f32)


def _lhs7(a, b, c, d):
    return [a + d, c + d, a, d, a + b, c - a, b - d]


def _rhs7(a, b, c, d):
    return [a + d, a, b - d, c - a, d, a + b, c + d]


_USES = (((0, 1), (3, 1)), ((2, 1), (3, -1)), ((1, 1), (3, 1)), ((0, 1), (2, 1)),
         ((0, -1), (1, 1)), ((3, 1),), ((0, 1),))
_LAST = (6, 4, 3, 5)


def _forms49(f, x):
    outer = [f(x[r][c], x[r][2 + c], x[2 + r][c], x[2 + r][2 + c])
             for r in range(2) for c in range(2)]
    return [y for g in range(7) for y in f(*[o[g] for o in outer])]


def _lhs49(even, odd):
    return [_pack2(a, b) for a, b in zip(_forms49(_lhs7, even), _forms49(_lhs7, odd))]


def _rhs49(even, odd, words):
    plain = {8: words[0][0], 11: words[1][1], 29: words[2][2], 32: words[3][3]}
    forms = zip(_forms49(_rhs7, even), _forms49(_rhs7, odd))
    return [plain[p] if p in plain else _pack2(a, b) for p, (a, b) in enumerate(forms)]


def _rhs49_words(words):
    return _rhs49([[_half(w, 0) for w in row] for row in words],
                  [[_half(w, 1) for w in row] for row in words], words)


def _products49(product, emit, start=None, between=None):
    def add(acc, v, sign):
        if acc is None:
            return v
        return acc + v if sign > 0 else acc - v

    total = {}
    for g in range(7):
        inner = [None] * 4
        for e in range(7):
            m = product(7 * g + e)
            for q, sign in _USES[e]:
                inner[q] = add(inner[q], m, sign)
            for q in range(4):
                if e != _LAST[q]:
                    continue
                for o, sign in _USES[g]:
                    rc = (2 * (o // 2) + q // 2, 2 * (o % 2) + q % 2)
                    if rc not in total and start is not None:
                        total[rc] = start(*rc)
                    total[rc] = add(total.get(rc), inner[q], sign)
                    if g == _LAST[o]:
                        emit(*rc, total.pop(rc))
            if between is not None:
                between(7 * g + e)


def _kernel(x_hbm, mem0_ref, wq_hbm, wk_hbm, wv_hbm, wo_hbm, w1_hbm, w2_hbm,
            w3_hbm, w4_hbm, out_hbm,
            wo_b, hbuf, xg, w1b, w2b, w3b, w4b, sems, *q_rings):
    pl.run_scoped(
        functools.partial(_block_a, x_hbm, mem0_ref, (wq_hbm, wk_hbm, wv_hbm), wo_hbm,
                          w1_hbm, (w2_hbm, w3_hbm, w4_hbm), wo_b, hbuf, xg, w1b,
                          (w2b, w3b, w4b), sems, q_rings),
        [pltpu.VMEM((H, D // 2, DH), u32)] * 3,
        [pltpu.VMEM((H // 8, RING, DH), f32)] * 16,
        pltpu.VMEM((2 * TOK, D), u32),
    )
    pl.run_scoped(
        functools.partial(_block_b, (w2_hbm, w3_hbm, w4_hbm), out_hbm, wo_b, hbuf, xg,
                          w1b, (w2b, w3b, w4b), sems, q_rings),
        pltpu.VMEM((49, D // 8, C4), u32),
        pltpu.VMEM((F // FC, 49, D // 8, 128), u32),
        pltpu.VMEM((49, F // 8, C4), u32),
        pltpu.VMEM((49, RB // 8, C4), u32),
        pltpu.VMEM((D // 128, RB, 128), f32),
        pltpu.VMEM((S, D), bf16),
    )


def _late_copies(w_hbm, w_b, sems):
    return [pltpu.make_async_copy(src.bitcast(u32), dst, sems.at[SEM_W2 + i])
            for i, (src, dst) in enumerate(zip(w_hbm, w_b))]


def _block_a(x_hbm, mem0_ref, w_hbm, wo_hbm, w1_hbm, late_hbm, wo_b, hbuf, xg, w1b,
             late_b, sems, q_rings, w_s, kv_rings, ubuf):
    rings = list(q_rings) + list(kv_rings)
    ring = [[rings[m * 8 + h % 8].at[h // 8] for h in range(H)] for m in range(3)]
    q_r, k_r, v_r = ring

    def wo_copy(i):
        rows = pl.ds(_mult(i * 512, 512), 512)
        return pltpu.make_async_copy(wo_hbm.bitcast(u32).at[rows], wo_b.at[rows],
                                     sems.at[SEM_WO + i])

    def w1_copy(i):
        cols = pl.ds(_mult(i * C4, C4), C4)
        return pltpu.make_async_copy(w1_hbm.bitcast(u32).at[:, cols], w1b.at[i],
                                     sems.at[SEM_W1 + i])

    def prologue(stg, forms, x49, xs):
        x0_copy = pltpu.make_async_copy(x_hbm.at[pl.ds(0, P0)], xs.at[pl.ds(0, P0)],
                                        sems.at[SEM_X0])

        def x_copy(g):
            rows = pl.ds(_mult(P0 + g * 3 * XP, XP), 3 * XP)
            return pltpu.make_async_copy(x_hbm.at[rows], xs.at[rows], sems.at[SEM_X + g])

        def start_chunk(g, m):
            src = w_hbm[m].bitcast(u32)
            dst = stg[m].reshape(D // 2, 8, DH)
            for par in range(2):
                pltpu.make_async_copy(
                    src.at[:, pl.ds(_mult(16 * par + 4 * g, 4), 4), :],
                    dst.at[:, pl.ds(4 * par, 4), :],
                    sems.at[SEM_W + 3 * g + m]).start()

        def wait_chunk(g, m):
            pltpu.make_async_copy(stg[m], stg[m], sems.at[SEM_W + 3 * g + m]).wait()

        def relayout(g, m, half, i0):
            even, odd, words = [], [], []
            for k in range(4):
                i = k * (D // 8) + i0
                ev, od = [[stg[m][pl.ds(8 * i + 4 * par + 2 * half + a, 8, stride=8), :]
                           for a in range(2)] for par in range(2)]
                even.append([_half(ev[n // 2], n % 2) for n in range(4)])
                odd.append([_half(od[n // 2], n % 2) for n in range(4)])
                words.append([_pack2(a, b) for a, b in zip(even[k], odd[k])])
                for n in range(4):
                    w_s[m][8 * g + 4 * half + n, pl.ds(i, 8), :] = words[k][n]
            for p, v in enumerate(_rhs49(even, odd, words)):
                forms[half][p, pl.ds(i0, 8), :] = v

        def norm_rows(r0, n):
            xv = xs[pl.ds(r0, n), :].astype(f32)
            hbuf[pl.ds(r0, n), :] = xv
            xn = _ln(xv)
            for c in range(D // 128):
                xg[c, pl.ds(HALO + r0, n), :] = xn[:, c * 128:(c + 1) * 128]

        x0_copy.start()
        start_chunk(0, 0)
        x_copy(0).start()
        start_chunk(0, 1)
        start_chunk(0, 2)
        zero = jnp.zeros((HALO, 128), f32)
        for c in range(D // 128):
            xg[c, pl.ds(0, HALO), :] = zero
            xg[c, pl.ds(HALO + S, HALO), :] = zero
        x0_copy.wait()

        @pl.loop(0, P0 // 128)
        def _(i):
            norm_rows(pl.multiple_of(i * 128, 128), 128)

        @pl.loop(0, P0 // 64)
        def _(i):
            for c in range(2):
                even, odd = [[[xg[2 * k + c, pl.ds(HALO + a * (P0 // 4) + 16 * i + z, 8, stride=2), :]
                               for k in range(4)] for a in range(4)] for z in range(2)]
                for p, v in enumerate(_lhs49(even, odd)):
                    x49[p, pl.ds(pl.multiple_of(8 * i, 8), 8), pl.ds(128 * c, 128)] = v

        wait_chunk(0, 0)

        @pl.loop(0, D // 64)
        def _(i):
            relayout(0, 0, 0, pl.multiple_of(8 * i, 8))

        def stage(g, m, half):
            c = 3 * g + m
            if half == 0:
                g1, m1 = g, m
            else:
                g1, m1 = jnp.minimum(g + (1 if m == 2 else 0), 3), (m + 1) % 3
                pl.when(c < 11)(functools.partial(wait_chunk, g1, m1))
                if m == 0:
                    x_copy(g).wait()

                @pl.when(g < 3)
                def _():
                    start_chunk(g + 1, m)
                    if m == 0:
                        x_copy(g + 1).start()
                if m == 1:
                    wo_copy(g).start()
                if m == 2:
                    w1_copy(g).start()

            def product(p):
                return _dot(_unpack(x49[p]), _unpack(forms[half][p]))

            def emit(a, n, v):
                rings[m * 8 + 4 * half + n][g, pl.ds(a * (P0 // 4), P0 // 4), :] = v

            def between(p):
                if p % 3 == 0 and p < 48:
                    relayout(g1, m1, 1 - half, 8 * (p // 3))
                if half == 1 and p % 6 == 1 and p < 48:
                    norm_rows(pl.multiple_of(P0 + c * XP + 16 * (p // 6), 16), 16)

            _products49(product, emit, between=between)

        @pl.loop(0, 4)
        def _(g):
            for m in range(3):
                for half in range(2):
                    stage(g, m, half)

    pl.run_scoped(
        prologue,
        [pltpu.VMEM((8 * D // 2, DH), u32)] * 3,
        [pltpu.VMEM((49, D // 8, DH), u32)] * 2,
        pltpu.VMEM((49, P0 // 8, C4), u32),
        pltpu.VMEM((S, D), bf16),
    )
    for copy in _late_copies(late_hbm, late_b, sems):
        copy.start()
    for i in range(4):
        wo_copy(i).wait()
    for i in range(4):
        w1_copy(i).wait()

    def wrap(r):
        return jnp.where(r >= RING, r - RING, r)

    def load_tok(s):
        rows = pl.ds(pl.multiple_of(HALO + P0 + TOK * s, 8), TOK)
        return jnp.concatenate([xg[c, rows, :] for c in range(D // 128)], axis=1)

    def step(s, carry, tok, first_of_group):
        mem, rp, ra, rw = carry
        ri = lax.broadcasted_iota(jnp.int32, (L, L), 0)
        ci = lax.broadcasted_iota(jnp.int32, (L, L), 1)
        mask = (ri < MEM) | (ri >= ci)

        lhs = jnp.concatenate([mem, tok], axis=0).astype(bf16)
        rps = [pl.multiple_of(wrap(rp + 8 * i), 8) for i in range(3)]
        ra_ = pl.multiple_of(ra, SEG)
        rw_ = pl.multiple_of(rw, 8)

        col = s & 3
        rb = pl.multiple_of(jnp.maximum((s >> 2) - 1, 0) * (4 * TOK), 8)
        if first_of_group:
            ubuf[...] = _pack(_ln(_ln(hbuf[pl.ds(rb, 4 * TOK), :])))

        def filler(j):
            r = _dot(_unpack(ubuf[...]), _unpack(w1b[col, :, pl.ds(j * 128, 128)]))
            xg[2 * col + j, pl.ds(HALO + rb, 4 * TOK), :] = _gelu(r)

        mem_qkv = {}
        scores = {}
        o_mem = {}
        total = [None]

        def qkv(h):
            res = []
            for m in range(3):
                r = _dot(lhs, _unpack(w_s[m][h]))
                for i in range(3):
                    ring[m][h][pl.ds(rps[i], 8), :] = r[8 + 8 * i:16 + 8 * i]
                res.append(r[:MEM])
            mem_qkv[h] = res

        def qk(h):
            qm, km, vm = mem_qkv.pop(h)
            qa = jnp.concatenate([qm, q_r[h][pl.ds(ra_, SEG), :]], axis=0).astype(bf16)
            ka = jnp.concatenate([km, k_r[h][pl.ds(ra_, SEG), :]], axis=0).astype(bf16)
            sc = lax.dot_general(qa, ka, (((1,), (1,)), ((), ())),
                                 preferred_element_type=f32)
            scores[h] = (sc, vm)

        def pv(h):
            sc, vm = scores.pop(h)
            va = jnp.concatenate([vm, v_r[h][pl.ds(ra_, SEG), :]], axis=0).astype(bf16)
            sc = jnp.where(mask, sc * (DH ** -0.5), NEG)
            mx = jnp.max(sc, axis=1, keepdims=True)
            e = jnp.exp(sc - mx)
            den = jnp.sum(e, axis=1, keepdims=True)
            inv = pl.reciprocal(den, approx=True)
            inv = inv * (2.0 - den * inv)
            o = _dot(e.astype(bf16), va) * inv
            q_r[h][pl.ds(ra_, SEG), :] = o[MEM:]
            o_mem[h] = o[:MEM]

        def wo(h):
            lo = jnp.concatenate([o_mem.pop(h), q_r[h][pl.ds(rw_, TOK), :]],
                                 axis=0).astype(bf16)
            r = _dot(lo, _unpack(wo_b[pl.ds(h * DH // 2, DH // 2), :]))
            total[0] = r if total[0] is None else total[0] + r

        npair = H // 2
        for t in range(npair + LAG_WO):
            if 0 <= t - LAG_QK < npair:
                qk(2 * (t - LAG_QK))
                qk(2 * (t - LAG_QK) + 1)
            if 0 <= t - LAG_PV < npair:
                pv(2 * (t - LAG_PV))
                pv(2 * (t - LAG_PV) + 1)
            if t < npair:
                qkv(2 * t)
                qkv(2 * t + 1)
            if t == FILL_AT:
                filler(0)
            if 0 <= t - LAG_WO < npair:
                wo(2 * (t - LAG_WO))
                wo(2 * (t - LAG_WO) + 1)
        filler(1)

        a = total[0]
        hbuf[pl.ds(pl.multiple_of(TOK * s, 8), TOK), :] += a[MEM:]
        return a[:MEM], wrap(rp + TOK), wrap(ra + SEG), wrap(rw + TOK)

    def steps(i, carry):
        toks = [load_tok(i * UNROLL + k) for k in range(UNROLL)]
        for k in range(UNROLL):
            carry = step(i * UNROLL + k, carry, toks[k], k == 0)
        return carry

    lax.fori_loop(
        0, NSEG // UNROLL, steps,
        (mem0_ref[...].astype(f32), jnp.int32(P0), jnp.int32(0), jnp.int32(0)))


def _block_b(late_hbm, out_hbm, wo_b, hbuf, xg, w1b, late_b, sems, q_rings,
             w2s, w3s, w4s, y49, ybuf, obuf):
    q_r = [q_rings[h % 8].at[h // 8] for h in range(H)]
    w2b, w3b, w4b = late_b
    for copy in _late_copies(late_hbm, late_b, sems):
        copy.wait()
    nj = F // FC
    Q = RB // 4

    def out_copy(i):
        rows = pl.ds(_mult(i * RB, RB), RB)
        return pltpu.make_async_copy(obuf.at[rows], out_hbm.at[rows], sems.at[SEM_OUT + i])

    def w2_piece(i, c):
        words = [[w2b[pl.ds(k * (D // 8) + i, 8), pl.ds(n * C4 + c, 128)]
                  for n in range(4)] for k in range(4)]
        for p, v in enumerate(_rhs49_words(words)):
            w2s[p, pl.ds(i, 8), pl.ds(c, 128)] = v

    def w3_piece(j, i):
        words = [[w3b[pl.ds(k * (D // 8) + i, 8), pl.ds(j * FC + n * 128, 128)]
                  for n in range(4)] for k in range(4)]
        for p, v in enumerate(_rhs49_words(words)):
            w3s[j, p, pl.ds(i, 8), :] = v

    def w4_piece(j, i, c):
        words = [[w4b[pl.ds(j * (FC // 2) + k * 64 + i, 8), pl.ds(n * C4 + c, 128)]
                  for n in range(4)] for k in range(4)]
        for p, v in enumerate(_rhs49_words(words)):
            w4s[p, pl.ds(j * 64 + i, 8), pl.ds(c, 128)] = v

    def wo_batch(r0, n):
        rr = r0 % RING
        lo = jnp.concatenate(
            [q_r[h][pl.ds(rr, n), :].astype(bf16) for h in range(H)], axis=1)
        hbuf[pl.ds(r0, n), :] += _dot(lo, _unpack(wo_b[...]))

    def mixer_norm(r0, n):
        return _ln(_ln(hbuf[pl.ds(r0, n), :])).astype(bf16)

    def mixer_in(r0, u):
        for c in range(4):
            g = _gelu(_dot(u, _unpack(w1b[c])))
            for j in range(2):
                xg[2 * c + j, pl.ds(HALO + r0, u.shape[0]), :] = g[:, j * 128:(j + 1) * 128]

    def mixer_out(i):
        r0 = i * RB
        pieces = {}
        for r in range(0, Q, 16):
            for c in range(2):
                even, odd = [[[xg[2 * k + c, pl.ds(HALO + r0 + a * Q + r + off + z, 8, stride=2), :]
                               for k, off in enumerate((-1, 1, -2, 2))]
                              for a in range(4)] for z in range(2)]
                pieces[r, c] = _lhs49(even, odd)

        def product(p):
            g = jnp.concatenate(
                [jnp.concatenate([pieces[r, c][p] for r in range(0, Q, 16)], axis=0)
                 for c in range(2)], axis=1)
            return _dot(_unpack(g), _unpack(w2s[p]))

        hs = {}

        def emit(a, n, v):
            hs[a, n] = v
            if all((a, k) in hs for k in range(4)):
                rows = pl.ds(_mult(r0 + a * Q, Q), Q)
                hv = hbuf[rows, :]
                x1 = _ln(hv) + jnp.concatenate([hs.pop((a, k)) for k in range(4)], axis=1)
                hbuf[rows, :] = hv + x1
                y = _ln(x1)
                for c in range(D // 128):
                    ybuf[c, pl.ds(a * Q, Q), :] = y[:, c * 128:(c + 1) * 128]

        _products49(product, emit)

    def y_piece(r, c):
        first = 32 * (r // 32) + (r // 16) % 2
        even, odd = [[[ybuf[2 * k + c, pl.ds(a * Q + first + 2 * z, 8, stride=4), :]
                       for k in range(4)] for a in range(4)] for z in range(2)]
        for p, v in enumerate(_lhs49(even, odd)):
            y49[p, pl.ds(r // 2, 8), pl.ds(128 * c, 128)] = v

    y_pieces = [(r, c) for r in range(0, Q, 16) for c in range(2)]

    def mlp_block(i, last):
        hidden = {}
        for j in range(nj):
            t = {}
            _products49(lambda p: _dot(_unpack(y49[p]), _unpack(w3s[j, p])),
                        lambda a, n, v: t.__setitem__((a, n), _gelu(v)))
            for r in range(0, Q, 16):
                first = 32 * (r // 32) + 8 * ((r // 16) % 2)
                even, odd = [[[t[a, n][first + 16 * z:first + 16 * z + 8] for n in range(4)]
                              for a in range(4)] for z in range(2)]
                hidden[j, r] = _lhs49(even, odd)

        def down(p, j0, j1):
            lhs = jnp.concatenate(
                [jnp.concatenate([hidden[j, r][p] for r in range(0, Q, 16)], axis=0)
                 for j in range(j0, j1)], axis=1)
            return _dot(_unpack(lhs), _unpack(w4s[p, pl.ds(64 * j0, 64 * (j1 - j0)), :]))

        if last:
            early = {p: down(p, 0, nj - 1) for p in range(EARLY)}
        else:
            early = {}
            mixer_out(i + 1)

        def product(p):
            return early.pop(p) + down(p, nj - 1, nj) if p in early else down(p, 0, nj)

        def rows(a):
            return pl.ds(_mult(i * RB + a * Q, Q), Q)

        def emit(a, n, v):
            obuf[rows(a), pl.ds(n * C4, C4)] = v.astype(bf16)

        def between(p):
            if not last and p >= 16 and p % 2 == 0 and (p - 16) // 2 < len(y_pieces):
                y_piece(*y_pieces[(p - 16) // 2])

        _products49(product, emit, lambda a, n: hbuf[rows(a), pl.ds(n * C4, C4)], between)
        out_copy(i).start()

    done = TOK * NSEG
    split = 3 * RING
    first = 4 * TOK * (NSEG // 4 - 1)
    for i in range(0, D // 8, 8):
        for c in range(0, C4, 128):
            w2_piece(i, c)
    u = mixer_norm(first, done - first)
    wo_batch(done, split - done)
    mixer_in(first, u)
    mixer_out(0)
    for j in range(nj):
        for i in range(0, D // 8, 8):
            w3_piece(j, i)
    u = mixer_norm(done, split - done)
    wo_batch(split, S - split)
    for piece in y_pieces:
        y_piece(*piece)
    for j in range(nj):
        for i in range(0, 64, 8):
            for c in range(0, C4, 128):
                w4_piece(j, i, c)
    mixer_in(done, u)
    mixer_in(split, mixer_norm(split, S - split))

    @pl.loop(0, S // RB - 1)
    def _(i):
        mlp_block(i, False)

    mlp_block(S // RB - 1, True)
    for i in range(S // RB):
        out_copy(i).wait()


@jax.jit
def pallas_sequential_preLN__memory_aug_recurrent_mem_tr__mixer_s_mlp__prompt_kernel(
    A_x: jax.Array,
    A_mem0: jax.Array,
    A_Wq: jax.Array,
    A_Wk: jax.Array,
    A_Wv: jax.Array,
    A_Wo: jax.Array,
    A_seg_len: jax.Array,
    B_x: jax.Array,
    B_w1: jax.Array,
    B_w2: jax.Array,
    B_w3: jax.Array,
    B_w4: jax.Array,
):
    del A_seg_len, B_x
    hbm = pl.BlockSpec(memory_space=pl.ANY)
    vmem = pl.BlockSpec(memory_space=pltpu.VMEM)
    scratch = [
        pltpu.VMEM((H * DH // 2, D), u32),
        pltpu.VMEM((S, D), f32),
        pltpu.VMEM((D // 128, S + 2 * HALO, 128), f32),
        pltpu.VMEM((4, D // 2, C4), u32),
        pltpu.VMEM((D // 2, D), u32),
        pltpu.VMEM((D // 2, F), u32),
        pltpu.VMEM((F // 2, D), u32),
        pltpu.SemaphoreType.DMA((NSEM,)),
    ] + [pltpu.VMEM((H // 8, RING, DH), f32)] * 8
    out = pl.pallas_call(
        _kernel,
        out_shape=jax.ShapeDtypeStruct((S, D), A_x.dtype),
        in_specs=[hbm, vmem] + [hbm] * 8,
        out_specs=hbm,
        scratch_shapes=scratch,
        compiler_params=pltpu.CompilerParams(vmem_limit_bytes=126 * 1024 * 1024),
    )(A_x.reshape(S, D), A_mem0.reshape(MEM, D),
      A_Wq.reshape(D // 2, 2 * H, DH), A_Wk.reshape(D // 2, 2 * H, DH),
      A_Wv.reshape(D // 2, 2 * H, DH),
      A_Wo.reshape(H * DH, D), B_w1, B_w2, B_w3, B_w4)
    return out.reshape(A_x.shape)
```

```python
import functools

import jax
import jax.numpy as jnp
from jax import lax
import jax.experimental.pallas as pl
import jax.experimental.pallas.tpu as pltpu

S = 2048
D = 1024
H = 32
DH = 128
MEM = 8
SEG = 32
F = 3584
NSEG = S // SEG
L = MEM + SEG
TOK = 24
P0 = S - TOK * NSEG
RING = 576
C4 = D // 4
HALO = 8
RB = 256
FC = 512
EPS = 1e-5
NEG = -1000000000.0

ORDER = "spbafxy"
LAG_QK = 2
LAG_PV = 4
LAG_WO = 5
FILL_AT = (4, 0)
G_FROM = 68
G_TO = 96
TK = 512
TQ = 4
TEND = 4
UQ = 4
UN = 8
ULEAD = 32
LN_ROWS = 8
LN_GAP = 3
Y_FROM = 38
Y_TO = 68
TM = 128
UM = 128
DW = 128
MW = 128
FLAG = 0
EARLY = 16
PSUB = 2
FENCE = 0
DMA_AT = (0, 2, 4, 6, 8, 8, 8, 8, 9)
PLAIN = 1
RG = 4
PEND = 2
UNROLL = 2

bf16 = jnp.bfloat16
f32 = jnp.float32
u32 = jnp.uint32

SEM_X0, SEM_X, SEM_WO, SEM_W1, SEM_W2, SEM_W3, SEM_W4, SEM_OUT, SEM_W = (
    0, 1, 5, 9, 13, 14, 15, 16, 32)
NSEM = SEM_W + 12


def _mult(i, n):
    return i if isinstance(i, int) else pl.multiple_of(i, n)


def _ln(x):
    m = jnp.mean(x, axis=-1, keepdims=True)
    d = x - m
    v = jnp.mean(d * d, axis=-1, keepdims=True)
    return d * lax.rsqrt(v + EPS)


def _ln_twice(x, stats, rows):
    m = jnp.mean(x, axis=-1, keepdims=True)
    d = x - m
    scale = lax.rsqrt(jnp.mean(d * d, axis=-1, keepdims=True) + EPS)
    for k, v in enumerate((m, scale)):
        stats[k, rows, :] = jnp.broadcast_to(v, (x.shape[0], 128))
    return _ln(d * scale)


def _gelu(x):
    return jax.nn.gelu(x, approximate=True)


def _pack(x):
    return pltpu.bitcast(x.astype(bf16), u32)


def _unpack(x):
    return pltpu.bitcast(x, bf16)


def _pack2(even, odd):
    return pltpu.pack_elementwise([even, odd], packed_dtype=bf16)


def _half(w, i):
    return pltpu.unpack_elementwise(w, index=i, packed_dtype=bf16, unpacked_dtype=f32)


def _dot(a, b):
    return jnp.dot(a, b, preferred_element_type=f32)


_LHS = ((2, -1, 0), (2, 1, 3), (3, 0, None), (0, 1, 3), (0, 0, None), (0, 1, 1), (1, -1, 3))
_RHS = ((0, 1, 1), (0, 0, None), (2, -1, 0), (0, 1, 3), (1, -1, 3), (3, 0, None), (2, 1, 3))
_USES = (((3, 1),), ((2, 1), (3, -1)), ((2, 1), (0, 1)), ((0, 1), (3, 1)),
         ((3, 1), (1, 1)), ((1, 1), (0, -1)), ((0, 1),))
_LAST = (6, 5, 2, 4)
_PLAIN = (8, 12, 36, 40)


def _operands(table, g, block):
    def halves(x):
        return x if isinstance(x, (list, tuple)) else [_half(x, 0), _half(x, 1)]

    def comb(x, sign, y):
        return [a + b if sign > 0 else a - b for a, b in zip(halves(x), halves(y))]

    i, sign, j = table[g]
    inner = []
    for r in range(2):
        for c in range(2):
            x = block(2 * (i // 2) + r, 2 * (i % 2) + c)
            inner.append(comb(x, sign, block(2 * (j // 2) + r, 2 * (j % 2) + c)) if sign else x)
    out = []
    for i, sign, j in table:
        x = comb(inner[i], sign, inner[j]) if sign else inner[i]
        out.append(_pack2(*x) if isinstance(x, (list, tuple)) else x)
    return out


def _spread(works, steps, first, last, before=None, after=None):
    work = (v for w in works for v in w)
    total, n = steps * len(works), last - first

    def hook(t, result):
        if first <= t < last:
            count = (t + 1 - first) * total // n - (t - first) * total // n
            for k in range(count):
                if before is not None:
                    r = k * result.shape[0] // (8 * count) * 8
                    before(result[r:r + 8, :128])
                v = next(work)
                if after is not None:
                    after(v)
    return hook


def _tie(zero, *refs):
    def write(v):
        for ref in refs:
            rows = pl.ds(pl.multiple_of(ref.shape[-2] - 8 + 8 * zero, 8), 8)
            ref[(zero,) * (len(ref.shape) - 2) + (rows, pl.ds(0, 128))] = pltpu.bitcast(v, ref.dtype)
    return write


def _products49(product, emit, start=None, hooks=(), t0=0):
    def add(acc, v, sign):
        if acc is None:
            return v
        return acc + v if sign > 0 else acc - v

    total = {}
    for g in range(7):
        inner = [None] * 4
        for e in range(7):
            m = product(7 * g + e)
            for q, sign in _USES[e]:
                inner[q] = add(inner[q], m, sign)
            for q in range(4):
                if e != _LAST[q]:
                    continue
                for o, sign in _USES[g]:
                    rc = (2 * (o // 2) + q // 2, 2 * (o % 2) + q % 2)
                    if rc not in total and start is not None:
                        total[rc] = start(*rc)
                    total[rc] = add(total.get(rc), inner[q], sign)
                    if g == _LAST[o]:
                        emit(*rc, total.pop(rc))
            for hook in hooks:
                hook(t0 + 7 * g + e, m)


def _kernel(x_hbm, mem0_ref, wq_hbm, wk_hbm, wv_hbm, wo_hbm, w1_hbm, w2_hbm,
            w3_hbm, w4_hbm, out_hbm,
            wo_b, hbuf, xg, w1b, w2b, w3b, w4b, sems, zero_ref, stats, *q_rings):
    pl.run_scoped(
        functools.partial(_block_a, x_hbm, mem0_ref, (wq_hbm, wk_hbm, wv_hbm), wo_hbm,
                          w1_hbm, (w2_hbm, w3_hbm, w4_hbm), wo_b, hbuf, xg, w1b,
                          (w2b, w3b, w4b), sems, zero_ref, stats, q_rings),
        [pltpu.VMEM((H, D // 2, DH), u32)] * 3,
        [pltpu.VMEM((H // 8, RING, DH), f32)] * 16,
        pltpu.VMEM((2 * TOK, D), u32),
        pltpu.VMEM((S, D), bf16),
        pltpu.VMEM((UNROLL * TOK, D), f32),
        pltpu.SemaphoreType.REGULAR,
    )
    pl.run_scoped(
        functools.partial(_block_b, out_hbm, wo_b, hbuf, xg,
                          w1b, (w2b, w3b, w4b), sems, zero_ref, stats, q_rings),
        pltpu.VMEM((F // FC, 49, D // 8, 128), u32),
        pltpu.VMEM((49, D // 8, C4), u32),
        pltpu.VMEM((49, F // 8, C4), u32),
        pltpu.VMEM((49, RB // 8, C4), u32),
        pltpu.VMEM((49, RB // 8, C4), u32),
        pltpu.VMEM((RB + 8, D), f32),
        pltpu.VMEM((D // 128, RB + 8, 128), f32),
        pltpu.VMEM((2, RB, D), f32),
        pltpu.VMEM((2, RB, D), bf16),
    )


def _late_copies(w_hbm, w_b, sems):
    return [pltpu.make_async_copy(src.bitcast(u32), dst.at[pl.ds(0, dst.shape[0] - 8)],
                                  sems.at[SEM_W2 + i])
            for i, (src, dst) in enumerate(zip(w_hbm, w_b))]


def _block_a(x_hbm, mem0_ref, w_hbm, wo_hbm, w1_hbm, late_hbm, wo_b, hbuf, xg, w1b,
             late_b, sems, zero_ref, stats, q_rings, w_s, kv_rings, ubuf, xs, tokbuf, fence_sem):
    rings = list(q_rings) + list(kv_rings)
    ring = [[rings[m * 8 + h % 8].at[h // 8] for h in range(H)] for m in range(3)]
    q_r, k_r, v_r = ring

    def wo_copy(i):
        rows = pl.ds(i * 512, 512)
        return pltpu.make_async_copy(wo_hbm.bitcast(u32).at[rows], wo_b.at[rows],
                                     sems.at[SEM_WO + i])

    def w1_copy(i):
        cols = pl.ds(i * C4, C4)
        return pltpu.make_async_copy(w1_hbm.bitcast(u32).at[:, cols], w1b.at[i],
                                     sems.at[SEM_W1 + i])

    x_copies = [pltpu.make_async_copy(x_hbm.at[rows], xs.at[rows], sems.at[SEM_X + i])
                for i, rows in enumerate((pl.ds(0, P0), pl.ds(P0, S - P0)))]

    other_copies = [wo_copy(i) for i in range(4)] + [w1_copy(i) for i in range(4)] + x_copies[1:]

    def fence():
        pl.semaphore_signal(fence_sem, 1)
        pl.semaphore_wait(fence_sem, 1)

    def prologue(stg, forms, x49):
        def start_chunk(g, m):
            src = w_hbm[m].bitcast(u32)
            dst = stg[m].reshape(D // 2, 8, DH)
            for par in range(2):
                pltpu.make_async_copy(
                    src.at[:, pl.ds(_mult(16 * par + 4 * g, 4), 4), :],
                    dst.at[:, pl.ds(4 * par, 4), :],
                    sems.at[SEM_W + 3 * g + m]).start()

        def wait_chunk(g, m):
            pltpu.make_async_copy(stg[m], stg[m], sems.at[SEM_W + 3 * g + m]).wait()

        def relayout(g, m, half, i):
            for a in range(2):
                ev, od = [stg[m][pl.ds(8 * i + 4 * par + 2 * half + a, 8, stride=8), :]
                          for par in range(2)]
                for z in range(2):
                    w_s[m][8 * g + 4 * half + 2 * a + z, pl.ds(i, 8), :] = _pack2(
                        _half(ev, z), _half(od, z))

        def operands(g, m, half, i0):
            for k in range(4):
                relayout(g, m, half, k * (D // 8) + i0)
                yield
            for grp in range(7):
                def word(k, n):
                    return w_s[m][8 * g + 4 * half + n + (g >> (4 + grp // RG)),
                                  pl.ds(k * (D // 8) + i0, 8), :]
                for e, v in enumerate(_operands(_RHS, grp, word)):
                    if not (PLAIN and 7 * grp + e in _PLAIN):
                        forms[half + (g >> 2), 7 * grp + e, pl.ds(i0, 8), :] = v
                yield

        x_copies[0].start()
        for m in range(3):
            start_chunk(0, m)
        zero = jnp.zeros((HALO, 128), f32)
        for c in range(D // 128):
            xg[c, pl.ds(0, HALO), :] = zero
            xg[c, pl.ds(HALO + S, HALO), :] = zero
        x_copies[0].wait()

        @pl.loop(0, P0 // 128)
        def _(i):
            r0 = pl.multiple_of(i * 128, 128)
            xn = _ln(xs[pl.ds(r0, 128), :].astype(f32))
            for c in range(D // 128):
                xg[c, pl.ds(HALO + r0, 128), :] = xn[:, c * 128:(c + 1) * 128]

        @pl.loop(0, P0 // 64)
        def _(i):
            for c in range(2):
                def block(a, k):
                    return [xg[2 * k + c, pl.ds(HALO + a * (P0 // 4) + 16 * i + z, 8, stride=2), :]
                            for z in range(2)]
                for grp in range(7):
                    for e, v in enumerate(_operands(_LHS, grp, block)):
                        x49[7 * grp + e, pl.ds(pl.multiple_of(8 * i, 8), 8), pl.ds(128 * c, 128)] = v

        wait_chunk(0, 0)

        @pl.loop(0, D // 64)
        def _(i):
            for _ in operands(0, 0, 0, pl.multiple_of(8 * i, 8)):
                pass

        def stage(g, m, half):
            c = 3 * g + m
            if half == 0:
                g1, m1 = g, m
            else:
                g1, m1 = jnp.minimum(g + (1 if m == 2 else 0), 3), (m + 1) % 3
                pl.when(g < 3)(functools.partial(start_chunk, g + 1, m))
                for at, copy in zip(DMA_AT, other_copies):
                    if at % 3 == m:
                        pl.when(g == at // 3)(copy.start)
                pl.when(c < 11)(functools.partial(wait_chunk, g1, m1))
            if half == 0 and m > 0 and FENCE:
                fence()

            hook = _spread([operands(g1, m1, 1 - half, i0) for i0 in range(0, D // 8, 8)],
                           11, 0, 49 * PSUB - PEND)
            rows = P0 // 4 // PSUB
            for sub in range(PSUB):
                zero = g >> (3 + sub + PSUB * (2 * m + half))

                def product(p):
                    if PLAIN and p in _PLAIN:
                        k = _PLAIN.index(p)
                        w = w_s[m][8 * g + 4 * half + k + zero, pl.ds(k * (D // 8), D // 8), :]
                    else:
                        w = forms[half + zero, p]
                    return _dot(_unpack(x49[p + zero, pl.ds(sub * rows // 2, rows // 2), :]),
                                _unpack(w))

                def emit(a, n, v):
                    rings[m * 8 + 4 * half + n][g, pl.ds(a * (P0 // 4) + sub * rows, rows), :] = v

                _products49(product, emit, hooks=[hook], t0=49 * sub)

        @pl.loop(0, 4)
        def _(g):
            for m in range(3):
                for half in range(2):
                    stage(g, m, half)

    pl.run_scoped(
        prologue,
        [pltpu.VMEM((8 * D // 2, DH), u32)] * 3,
        pltpu.VMEM((2, 49, D // 8, DH), u32),
        pltpu.VMEM((49, P0 // 8, C4), u32),
    )
    for copy in _late_copies(late_hbm, late_b, sems):
        copy.start()
    for pending in other_copies:
        pending.wait()

    def wrap(r):
        return jnp.where(r >= RING, r - RING, r)

    def stage_tokens(i):
        n = UNROLL * TOK
        tokbuf[...] = _ln(xs[pl.ds(_mult(P0 + n * i, 16), n), :].astype(f32))

    def step(s, carry, tok, resid, first_of_group):
        mem, rp, ra, rw = carry
        ri = lax.broadcasted_iota(jnp.int32, (2 * L, 2 * L), 0)
        ci = lax.broadcasted_iota(jnp.int32, (2 * L, 2 * L), 1)
        same = (ri >= L) == (ci >= L)
        mask = same & ((jnp.where(ri >= L, ri - L, ri) < MEM) | (ri >= ci))
        fill = jnp.where(same, NEG, -jnp.inf)

        lhs = jnp.concatenate([mem, tok], axis=0).astype(bf16)
        rps = [pl.multiple_of(wrap(rp + 8 * i), 8) for i in range(3)]
        ra_ = pl.multiple_of(ra, SEG)
        rw_ = pl.multiple_of(rw, 8)

        col = s & 3
        rb = pl.multiple_of(jnp.maximum((s >> 2) - 1, 0) * (4 * TOK), 8)
        if first_of_group:
            ubuf[...] = _pack(_ln_twice(hbuf[pl.ds(rb, 4 * TOK), :], stats, pl.ds(rb, 4 * TOK)))

        def filler(j):
            r = _dot(_unpack(ubuf[...]), _unpack(w1b[col, :, pl.ds(j * 128, 128)]))
            xg[2 * col + j, pl.ds(HALO + rb, 4 * TOK), :] = _gelu(r)

        mem_qkv = {}
        scores = {}
        o_mem = {}
        total = [None]

        def qkv(h):
            res = []
            for m in range(3):
                r = _dot(lhs, _unpack(w_s[m][h]))
                for i in range(3):
                    ring[m][h][pl.ds(rps[i], 8), :] = r[8 + 8 * i:16 + 8 * i]
                res.append(r[:MEM])
            mem_qkv[h] = res

        def both(h, mem_rows, ring_m):
            return jnp.concatenate(
                [x for k in range(2) for x in (mem_rows[k], ring_m[h + k][pl.ds(ra_, SEG), :])],
                axis=0).astype(bf16)

        def qk(h):
            qm, km, vm = zip(mem_qkv.pop(h), mem_qkv.pop(h + 1))
            sc = lax.dot_general(both(h, qm, q_r), both(h, km, k_r), (((1,), (1,)), ((), ())),
                                 preferred_element_type=f32)
            scores[h] = (sc, vm)

        def pv(h):
            sc, vm = scores.pop(h)
            sc = jnp.where(mask, sc * (DH ** -0.5), fill)
            mx = jnp.max(sc, axis=1, keepdims=True)
            e = jnp.exp(sc - mx)
            den = jnp.sum(e, axis=1, keepdims=True)
            inv = pl.reciprocal(den, approx=True)
            inv = inv * (2.0 - den * inv)
            o = _dot(e.astype(bf16), both(h, vm, v_r)) * inv
            for k in range(2):
                q_r[h + k][pl.ds(ra_, SEG), :] = o[k * L + MEM:(k + 1) * L]
                o_mem[h + k] = o[k * L:k * L + MEM]

        def wo(h):
            lo = jnp.concatenate([o_mem.pop(h), q_r[h][pl.ds(rw_, TOK), :]],
                                 axis=0).astype(bf16)
            r = _dot(lo, _unpack(wo_b[pl.ds(h * DH // 2, DH // 2), :]))
            total[0] = r if total[0] is None else total[0] + r

        slot = {"s": (LAG_QK, qk, 0), "p": (LAG_PV, pv, 0), "a": (0, qkv, 0), "b": (0, qkv, 1),
                "x": (LAG_WO, wo, 0), "y": (LAG_WO, wo, 1)}
        for t in range(H // 2 + LAG_WO + 1):
            for kind in ORDER:
                if kind == "f":
                    for j in range(2):
                        if t == H // 2 + LAG_WO - FILL_AT[j]:
                            filler(j)
                    continue
                lag, fn, k = slot[kind]
                if 0 <= t - lag < H // 2:
                    fn(2 * (t - lag) + k)

        a = total[0]
        hbuf[pl.ds(pl.multiple_of(TOK * s, 8), TOK), :] = resid + a[MEM:]
        return a[:MEM], wrap(rp + TOK), wrap(ra + SEG), wrap(rw + TOK)

    def steps(i, carry):
        @pl.when(i == NSEG // UNROLL // 2)
        def _():
            for copy in _late_copies(late_hbm, late_b, sems):
                copy.wait()

        n = UNROLL * TOK
        toks = tokbuf[...]
        resid = xs[pl.ds(pl.multiple_of(n * i, 16), n), :].astype(f32)
        for k in range(UNROLL):
            rows = slice(k * TOK, (k + 1) * TOK)
            carry = step(i * UNROLL + k, carry, toks[rows], resid[rows], k == 0)
            if k == 0:
                stage_tokens(jnp.minimum(i + 1, NSEG // UNROLL - 1))
        return carry

    hbuf[pl.ds(0, 4 * TOK), :] = jnp.zeros((4 * TOK, D), f32)
    hbuf[pl.ds(TOK * NSEG, P0), :] = xs[pl.ds(TOK * NSEG, P0), :].astype(f32)
    stage_tokens(0)
    carry = lax.fori_loop(
        0, NSEG // UNROLL, steps,
        (mem0_ref[...].astype(f32), jnp.int32(P0), jnp.int32(0), jnp.int32(0)))
    zero_ref[0] = carry[1] >> 12


def _block_b(out_hbm, wo_b, hbuf, xg, w1b, late_b, sems, zero_ref, stats, q_rings,
             w3s, w2s, w4s, y49, g49, xbuf, ybuf, res, obuf):
    w2b, w3b, w4b = late_b
    nj = F // FC
    Q = RB // 4

    def out_copy(i):
        rows = pl.ds(_mult(i * RB, RB), RB)
        return pltpu.make_async_copy(obuf.at[i & 1], out_hbm.at[rows], sems.at[SEM_OUT + (i & 1)])

    def weight_work(src, dst, row, col, at):
        for grp in range(7):
            def word(k, n):
                return src[pl.ds(_mult(row(k), 8), 8), pl.ds(col(n), 128)]
            for e, v in enumerate(_operands(_RHS, grp, word)):
                dst[at(7 * grp + e)] = v
            yield v

    def w2_work(i, c):
        return weight_work(w2b, w2s, lambda k: k * (D // 8) + i, lambda n: n * C4 + c,
                           lambda p: (p, pl.ds(_mult(i, 8), 8), pl.ds(c, 128)))

    def w3_work(j, i):
        return weight_work(w3b, w3s, lambda k: k * (D // 8) + i, lambda n: j * FC + n * 128,
                           lambda p: (j, p, pl.ds(_mult(i, 8), 8)))

    def w4_work(j, i, c):
        return weight_work(w4b, w4s, lambda k: j * (FC // 2) + k * 64 + i, lambda n: n * C4 + c,
                           lambda p: (p, pl.ds(_mult(j * 64 + i, 8), 8), pl.ds(c, 128)))

    def gather(pieces, p, cols):
        return _unpack(jnp.concatenate(
            [jnp.concatenate([pieces[c, r][p] for r in range(0, Q, 16)], axis=0)
             for c in cols], axis=1))

    def left_work(dst, block, r, c):
        for grp in range(7):
            for e, v in enumerate(_operands(_LHS, grp, block)):
                dst[7 * grp + e, pl.ds(_mult(r // 2, 8), 8), pl.ds(128 * c, 128)] = v
            yield v

    def shift_work(i, r, c):
        def block(a, k):
            r0 = HALO + i * RB + a * Q + r + (-1, 1, -2, 2)[k]
            return [xg[2 * k + c, pl.ds(r0 + z, 8, stride=2), :] for z in range(2)]
        return left_work(g49, block, r, c)

    def y_work(r, c):
        def block(a, k):
            r0 = a * Q + 32 * (r // 32) + (r // 16) % 2
            return [ybuf[2 * k + c, pl.ds(r0 + 2 * z, 8, stride=4), :] for z in range(2)]
        return left_work(y49, block, r, c)

    pieces = [(r, c) for r in range(0, Q, 16) for c in range(2)]

    def mixer_out(i, hooks=()):
        for c in range(0, C4, MW):
            def emit(a, n, v):
                rows, cols = pl.ds(_mult(i * RB + a * Q, Q), Q), pl.ds(n * C4 + c, MW)
                hv = hbuf[rows, cols]
                mean, scale = [jnp.tile(stats[k, rows, :], (1, MW // 128)) for k in range(2)]
                x1 = (hv - mean) * scale + v
                xbuf[pl.ds(a * Q, Q), cols] = x1
                res[i & 1, pl.ds(a * Q, Q), cols] = hv + x1

            _products49(lambda p: _dot(_unpack(g49[p]), _unpack(w2s[p, :, pl.ds(c, MW)])),
                        emit, hooks=hooks, t0=49 * c // MW)

    def norm_x1(r):
        y = _ln(xbuf[pl.ds(r, LN_ROWS), :])
        for k in range(D // 128):
            ybuf[k, pl.ds(r, LN_ROWS), :] = y[:, k * 128:(k + 1) * 128]
        yield

    def post_hooks(zero, t0, t1, t2):
        return [_spread([norm_x1(r) for r in range(0, RB, LN_ROWS)], 1, t0, t1 - LN_GAP, _tie(zero, xbuf)),
                _spread([y_work(r, c) for r, c in pieces], 7, t1, t2, _tie(zero, ybuf))]

    def mlp_block(i, last):
        hidden = {}

        for j in range(nj):
            t = {}
            _products49(lambda p: _dot(_unpack(y49[p]), _unpack(w3s[j, p])),
                        lambda a, n, v: t.__setitem__((a, n), _gelu(v)))
            for r in range(0, Q, 16):
                r0 = 32 * (r // 32) + 8 * ((r // 16) % 2)
                hidden[j, r] = [v for grp in range(7) for v in _operands(
                    _LHS, grp, lambda a, n: [t[a, n][r0 + 16 * z:r0 + 16 * z + 8] for z in range(2)])]

        def down(p, c, j0, j1):
            return _dot(gather(hidden, p, range(j0, j1)),
                        _unpack(w4s[p, pl.ds(64 * j0, 64 * (j1 - j0)), pl.ds(c, DW)]))

        early = {(p, 0): down(p, 0, 0, nj - 1) for p in range(EARLY if last else 0)}
        hooks = []
        if not last:
            mixer_out(i + 1)
            ahead = jnp.minimum(i + 2, S // RB - 1)
            hooks = [_spread([shift_work(ahead, r, c) for r, c in pieces], 7, G_FROM, G_TO,
                             _tie(i >> 3, xg))]
            hooks += post_hooks(i >> 3, 0, Y_FROM, Y_TO)
        for c in range(0, C4, DW):
            def product(p):
                if (p, c) in early:
                    return early.pop((p, c)) + down(p, c, nj - 1, nj)
                return down(p, c, 0, nj)

            def emit(a, n, v):
                obuf[i & 1, pl.ds(a * Q, Q), pl.ds(n * C4 + c, DW)] = v.astype(bf16)

            _products49(product, emit,
                        lambda a, n: res[i & 1, pl.ds(a * Q, Q), pl.ds(n * C4 + c, DW)],
                        hooks, 49 * c // DW)
        out_copy(i).start()

    done = TOK * NSEG
    first = 4 * TOK * (NSEG // 4 - 1)

    @pl.loop(0, H // 8)
    def _(g):
        works = [[w2_work(32 * g + i, c) for i in range(0, 32, 8) for c in range(0, C4, 128)],
                 [shift_work(0, 16 * g, c) for c in range(2)],
                 [w3_work(j, 32 * g + i) for j in range(nj) for i in range(0, 32, 8)],
                 [w4_work(j, 16 * g + i, c) for j in range(nj)
                  for i in range(0, 16, 8) for c in range(0, C4, 128)]]
        per = TK // DH
        calls = P0 // TM * (8 // per) * 8 * TQ - TEND
        ends = [calls * sum(map(len, works[:k])) // sum(map(len, works)) for k in range(5)]
        hooks = [_spread(works[k], 7, ends[k], ends[k + 1], _tie(g >> 2, src))
                 for k, src in enumerate((w2b, xg, w3b, w4b))]
        t = 0
        for r0 in range(done, S, TM):
            rr = r0 % RING
            n = min(TM, RING - rr)
            spans = [(rr, n)] + ([(0, TM - n)] if n < TM else [])
            for k in range(0, 8, per):
                lo = jnp.concatenate(
                    [jnp.concatenate([q_rings[h][g, pl.ds(*span), :] for span in spans], axis=0)
                     for h in range(k, k + per)], axis=1).astype(bf16)
                rows = pl.ds(pl.multiple_of((8 * g + k) * (DH // 2), TK // 2), TK // 2)
                for c in range(0, D, 128):
                    r = _dot(lo, _unpack(wo_b[rows, pl.ds(c, 128)]))
                    for q in range(0, TM, TM // TQ):
                        hbuf[pl.ds(r0 + q, TM // TQ), pl.ds(c, 128)] += r[q:q + TM // TQ]
                        for hook in hooks:
                            hook(t, r[q:q + TM // TQ])
                        t += 1

    zero = zero_ref[0]
    us = {}

    def norm_h(r):
        us[r] = _ln_twice(hbuf[pl.ds(r, UN), :], stats, pl.ds(r, UN))
        yield

    blocks = [(first, done - first)] + [(r0, UM) for r0 in range(done, S, UM)]
    lead = 49 * C4 // MW
    calls = lead + 8 * UQ * len(blocks)
    hooks = [_spread([norm_h(r) for r in range(first, S, UN)], 1, 0, calls - 8 * UQ - ULEAD,
                     _tie(zero, hbuf)),
             _spread([shift_work(1, r, c) for r, c in pieces], 7, lead, calls - 1, _tie(zero, xg))]
    hooks += post_hooks(zero, lead, (lead + calls) // 2, calls - 1)
    mixer_out(0, hooks)
    for b, (r0, n) in enumerate(blocks):
        u = jnp.concatenate([us.pop(r) for r in range(r0, r0 + n, UN)], axis=0).astype(bf16)
        for c in range(D // 128):
            r = _dot(u, _unpack(w1b[c // 2, :, pl.ds(128 * (c % 2), 128)]))
            xg[c, pl.ds(HALO + r0, n), :] = _gelu(r)
            for q in range(UQ):
                for hook in hooks:
                    hook(lead + (8 * b + c) * UQ + q, r[q * n // UQ:(q + 1) * n // UQ])

    @pl.loop(0, S // RB - 1)
    def _(i):
        mlp_block(i, False)
        pl.when(i > 0)(lambda: out_copy(i - 1).wait())

    mlp_block(S // RB - 1, True)
    for i in range(S // RB - 2, S // RB):
        out_copy(i).wait()


@jax.jit
def pallas_sequential_preLN__memory_aug_recurrent_mem_tr__mixer_s_mlp__prompt_kernel(
    A_x: jax.Array,
    A_mem0: jax.Array,
    A_Wq: jax.Array,
    A_Wk: jax.Array,
    A_Wv: jax.Array,
    A_Wo: jax.Array,
    A_seg_len: jax.Array,
    B_x: jax.Array,
    B_w1: jax.Array,
    B_w2: jax.Array,
    B_w3: jax.Array,
    B_w4: jax.Array,
):
    del A_seg_len, B_x
    hbm = pl.BlockSpec(memory_space=pl.ANY)
    vmem = pl.BlockSpec(memory_space=pltpu.VMEM)
    scratch = [
        pltpu.VMEM((H * DH // 2, D), u32),
        pltpu.VMEM((S + 8, D), f32),
        pltpu.VMEM((D // 128, S + 2 * HALO + 8, 128), f32),
        pltpu.VMEM((4, D // 2, C4), u32),
        pltpu.VMEM((D // 2 + 8, D), u32),
        pltpu.VMEM((D // 2 + 8, F), u32),
        pltpu.VMEM((F // 2 + 8, D), u32),
        pltpu.SemaphoreType.DMA((NSEM,)),
        pltpu.SMEM((1,), jnp.int32),
        pltpu.VMEM((2, S, 128), f32),
    ] + [pltpu.VMEM((H // 8, RING, DH), f32)] * 8
    out = pl.pallas_call(
        _kernel,
        out_shape=jax.ShapeDtypeStruct((S, D), A_x.dtype),
        in_specs=[hbm, vmem] + [hbm] * 8,
        out_specs=hbm,
        scratch_shapes=scratch,
        compiler_params=pltpu.CompilerParams(
            vmem_limit_bytes=127 * 1024 * 1024,
            flags=[None, {"XLA_TPU_FORCE_LP_LLO_SCHEDULER": True}, {"XLA_TPU_EVENLY_DISTRIBUTE_CRITICAL_NODES": True}][FLAG]),
    )(A_x.reshape(S, D), A_mem0.reshape(MEM, D),
      A_Wq.reshape(D // 2, 2 * H, DH), A_Wk.reshape(D // 2, 2 * H, DH),
      A_Wv.reshape(D // 2, 2 * H, DH),
      A_Wo.reshape(H * DH, D), B_w1, B_w2, B_w3, B_w4)
    return out.reshape(A_x.shape)
```

```python
import functools

import jax
import jax.numpy as jnp
from jax import lax
import jax.experimental.pallas as pl
import jax.experimental.pallas.tpu as pltpu

S = 2048
D = 1024
H = 32
DH = 128
MEM = 8
SEG = 32
F = 3584
NSEG = S // SEG
L = MEM + SEG
TOK = 24
P0 = S - TOK * NSEG
RING = 576
C4 = D // 4
HALO = 8
RB = 256
FC = 512
EPS = 1e-5
NEG = -1000000000.0

ORDER = "spbafxy"
LAG_QK = 2
LAG_PV = 4
LAG_WO = 6
FILL_AT = (4, 0)
G_FROM = 68
G_TO = 97
TK = 512
TQ = 8
TEND = 8
UQ = 2
UN = 8
ULEAD = 80
LN_ROWS = 8
LN_GAP = 2
Y_FROM = 38
Y_TO = 68
TM = 128
UM = 64
MW = 128
FLAG = 0
EARLY = 16
PSUB = 2
X_LATE = 704
DMA_AT = (2, 4, 6, 8, 9, 9, 9, 9, 9, 9)
RAT = (0, 1, 4, 5)
WAT = 1
PBEG = 1
RG = 2
PEND = 2
FILL_B = (4, 2)
UNROLL = 2

bf16 = jnp.bfloat16
f32 = jnp.float32
u32 = jnp.uint32

SEM_X, SEM_XR, SEM_WO, SEM_W1, SEM_W2, SEM_OUT, SEM_W0, SEM_W = 0, 4, 7, 11, 15, 18, 21, 22
NSEM = SEM_W + 12


def _mult(i, n):
    return i if isinstance(i, int) else pl.multiple_of(i, n)


def _ln(x):
    m = jnp.mean(x, axis=-1, keepdims=True)
    d = x - m
    v = jnp.mean(d * d, axis=-1, keepdims=True)
    return d * lax.rsqrt(v + EPS)


def _ln_twice(x, stats, rows):
    m = jnp.mean(x, axis=-1, keepdims=True)
    d = x - m
    scale = lax.rsqrt(jnp.mean(d * d, axis=-1, keepdims=True) + EPS)
    for k, v in enumerate((m, scale)):
        stats[k, rows, :] = jnp.broadcast_to(v, (x.shape[0], 128))
    return _ln(d * scale)


def _gelu(x):
    return jax.nn.gelu(x, approximate=True)


def _pack(x):
    return pltpu.bitcast(x.astype(bf16), u32)


def _unpack(x):
    return pltpu.bitcast(x, bf16)


def _pack2(even, odd):
    return pltpu.pack_elementwise([even, odd], packed_dtype=bf16)


def _half(w, i):
    return pltpu.unpack_elementwise(w, index=i, packed_dtype=bf16, unpacked_dtype=f32)


def _dot(a, b):
    return jnp.dot(a, b, preferred_element_type=f32)


_LHS = ((2, -1, 0), (2, 1, 3), (3, 0, None), (0, 1, 3), (0, 0, None), (0, 1, 1), (1, -1, 3))
_RHS = ((0, 1, 1), (0, 0, None), (2, -1, 0), (0, 1, 3), (1, -1, 3), (3, 0, None), (2, 1, 3))
_USES = (((3, 1),), ((2, 1), (3, -1)), ((2, 1), (0, 1)), ((0, 1), (3, 1)),
         ((3, 1), (1, 1)), ((1, 1), (0, -1)), ((0, 1),))
_LAST = (6, 5, 2, 4)
_PLAIN = (8, 12, 36, 40)


def _operands(table, g, block):
    def halves(x):
        return x if isinstance(x, (list, tuple)) else [_half(x, 0), _half(x, 1)]

    def comb(x, sign, y):
        return [a + b if sign > 0 else a - b for a, b in zip(halves(x), halves(y))]

    i, sign, j = table[g]
    inner = []
    for r in range(2):
        for c in range(2):
            x = block(2 * (i // 2) + r, 2 * (i % 2) + c)
            inner.append(comb(x, sign, block(2 * (j // 2) + r, 2 * (j % 2) + c)) if sign else x)
    out = []
    for i, sign, j in table:
        x = comb(inner[i], sign, inner[j]) if sign else inner[i]
        out.append(_pack2(*x) if isinstance(x, (list, tuple)) else x)
    return out


def _spread(works, steps, first, last, before=None, after=None):
    work = (v for w in works for v in w)
    total, n = steps * len(works), last - first

    def hook(t, result):
        if first <= t < last:
            count = (t + 1 - first) * total // n - (t - first) * total // n
            for k in range(count):
                if before is not None:
                    r = k * result.shape[0] // (8 * count) * 8
                    before(result[r:r + 8, :128])
                v = next(work)
                if after is not None:
                    after(v)
    return hook


def _tie(zero, *refs):
    def write(v):
        for ref in refs:
            rows = pl.ds(pl.multiple_of(ref.shape[-2] - 8 + 8 * zero, 8), 8)
            ref[(zero,) * (len(ref.shape) - 2) + (rows, pl.ds(0, 128))] = pltpu.bitcast(v, ref.dtype)
    return write


def _products49(product, emit, start=None, hooks=(), t0=0):
    def add(acc, v, sign):
        if acc is None:
            return v
        return acc + v if sign > 0 else acc - v

    total = {}
    for g in range(7):
        inner = [None] * 4
        for e in range(7):
            m = product(7 * g + e)
            for q, sign in _USES[e]:
                inner[q] = add(inner[q], m, sign)
            for q in range(4):
                if e != _LAST[q]:
                    continue
                for o, sign in _USES[g]:
                    rc = (2 * (o // 2) + q // 2, 2 * (o % 2) + q % 2)
                    if rc not in total and start is not None:
                        total[rc] = start(*rc)
                    total[rc] = add(total.get(rc), inner[q], sign)
                    if g == _LAST[o]:
                        emit(*rc, total.pop(rc))
            for hook in hooks:
                hook(t0 + 7 * g + e, m)


def _kernel(x_hbm, mem0_ref, wq_hbm, wk_hbm, wv_hbm, wo_hbm, w1_hbm, w2_hbm,
            w3_hbm, w4_hbm, out_hbm,
            wo_b, hbuf, xg, w1b, w2b, w3b, w4b, sems, zero_ref, stats, *q_rings):
    pl.run_scoped(
        functools.partial(_block_a, x_hbm, mem0_ref, (wq_hbm, wk_hbm, wv_hbm), wo_hbm,
                          w1_hbm, (w2_hbm, w3_hbm, w4_hbm), wo_b, hbuf, xg, w1b,
                          (w2b, w3b, w4b), sems, zero_ref, stats, q_rings),
        [pltpu.VMEM((H, D // 2, DH), u32)] * 3,
        [pltpu.VMEM((H // 8, RING, DH), f32)] * 16,
        pltpu.VMEM((2 * TOK, D), u32),
        pltpu.VMEM((S, D), bf16),
        pltpu.VMEM((UNROLL * TOK, D), f32),
    )
    pl.run_scoped(
        functools.partial(_block_b, out_hbm, wo_b, hbuf, xg,
                          w1b, (w2b, w3b, w4b), sems, zero_ref, stats, q_rings),
        pltpu.VMEM((F // FC, 49, D // 8, 128), u32),
        pltpu.VMEM((49, D // 8, C4), u32),
        pltpu.VMEM((49, F // 8, C4), u32),
        pltpu.VMEM((49, RB // 8, C4), u32),
        pltpu.VMEM((49, RB // 8, C4), u32),
        pltpu.VMEM((RB + 8, D), f32),
        pltpu.VMEM((D // 128, RB + 8, 128), f32),
        pltpu.VMEM((2, RB, D), f32),
        pltpu.VMEM((2, RB, D), bf16),
    )


def _late_copies(w_hbm, w_b, sems):
    return [pltpu.make_async_copy(src.bitcast(u32), dst.at[pl.ds(0, dst.shape[0] - 8)],
                                  sems.at[SEM_W2 + i])
            for i, (src, dst) in enumerate(zip(w_hbm, w_b))]


def _block_a(x_hbm, mem0_ref, w_hbm, wo_hbm, w1_hbm, late_hbm, wo_b, hbuf, xg, w1b,
             late_b, sems, zero_ref, stats, q_rings, w_s, kv_rings, ubuf, xs, tokbuf):
    rings = list(q_rings) + list(kv_rings)
    ring = [[rings[m * 8 + h % 8].at[h // 8] for h in range(H)] for m in range(3)]
    q_r, k_r, v_r = ring

    def wo_copy(i):
        rows = pl.ds(i * 512, 512)
        return pltpu.make_async_copy(wo_hbm.bitcast(u32).at[rows], wo_b.at[rows],
                                     sems.at[SEM_WO + i])

    def w1_copy(i):
        cols = pl.ds(i * C4, C4)
        return pltpu.make_async_copy(w1_hbm.bitcast(u32).at[:, cols], w1b.at[i],
                                     sems.at[SEM_W1 + i])

    x_rest = [pltpu.make_async_copy(x_hbm.at[pl.ds(r0, r1 - r0)], xs.at[pl.ds(r0, r1 - r0)],
                                    sems.at[SEM_XR + i])
              for i, (r0, r1) in enumerate(((P0, X_LATE), (S - P0, S), (X_LATE, S - P0)))]
    other_copies = [wo_copy(i) for i in range(4)] + [w1_copy(i) for i in range(4)] + x_rest[:2]

    def prologue(stg, forms, x49):
        def start_chunk(g, m, pairs=range(4), sem=None):
            for pair in pairs:
                pltpu.make_async_copy(
                    w_hbm[m].bitcast(u32).at[:, 4 * g + pair, :], stg[m].at[pl.ds(pair * D, D)],
                    sems.at[SEM_W + 3 * g + m if sem is None else sem]).start()

        def wait_chunk(g, m, rows=pl.ds(0, 4 * D), sem=None):
            pltpu.make_async_copy(stg[m].at[rows], stg[m].at[rows],
                                  sems.at[SEM_W + 3 * g + m if sem is None else sem]).wait()

        def relayout(g, m, half, i):
            for a in range(2):
                ev, od = [stg[m][pl.ds((2 * half + a) * D + 2 * i + par, 8, stride=2), :]
                          for par in range(2)]
                for z in range(2):
                    w_s[m][8 * g + 4 * half + 2 * a + z, pl.ds(i, 8), :] = _pack2(
                        _half(ev, z), _half(od, z))

        def operands(g, m, half, i0, ahead):
            for grp in range(7):
                def word(k, n):
                    return w_s[m][8 * g + 4 * half + n + (g >> (4 + grp // RG)),
                                  pl.ds(k * (D // 8) + i0, 8), :]
                for e, v in enumerate(_operands(_RHS, grp, word)):
                    if 7 * grp + e not in _PLAIN:
                        forms[half + (g >> 2), 7 * grp + e, pl.ds(i0, 8), :] = v
                        yield
                if ahead is not None and grp in RAT:
                    relayout(g, m, half, RAT.index(grp) * (D // 8) + ahead)

        def x_copy(i):
            rows = pl.ds(_mult(i * 128, 128), 128)
            return pltpu.make_async_copy(x_hbm.at[rows], xs.at[rows], sems.at[SEM_X + i])

        start_chunk(0, 0, range(2), SEM_W0)
        for i in range(P0 // 128):
            x_copy(i).start()
        start_chunk(0, 0, range(2, 4))
        for m in range(1, 3):
            start_chunk(0, m)
        zero = jnp.zeros((HALO, 128), f32)
        for c in range(D // 128):
            xg[c, pl.ds(0, HALO), :] = zero
            xg[c, pl.ds(HALO + S, HALO), :] = zero
        hbuf[pl.ds(0, 4 * TOK), :] = jnp.zeros((4 * TOK, D), f32)
        wait_chunk(0, 0, pl.ds(0, 2 * D), SEM_W0)

        @pl.loop(0, D // 64)
        def _(i):
            for k in range(4):
                relayout(0, 0, 0, pl.multiple_of(k * (D // 8) + 8 * i, 8))
            for _ in operands(0, 0, 0, pl.multiple_of(8 * i, 8), None):
                pass

        @pl.loop(0, P0 // 128)
        def _(i):
            x_copy(i).wait()
            r0 = pl.multiple_of(i * 128, 128)
            xn = _ln(xs[pl.ds(r0, 128), :].astype(f32))
            for c in range(D // 128):
                xg[c, pl.ds(HALO + r0, 128), :] = xn[:, c * 128:(c + 1) * 128]

        @pl.loop(0, P0 // 64)
        def _(i):
            for c in range(2):
                def block(a, k):
                    return [xg[2 * k + c, pl.ds(HALO + a * (P0 // 4) + 16 * i + z, 8, stride=2), :]
                            for z in range(2)]
                for grp in range(7):
                    for e, v in enumerate(_operands(_LHS, grp, block)):
                        x49[7 * grp + e, pl.ds(pl.multiple_of(8 * i, 8), 8), pl.ds(128 * c, 128)] = v

        wait_chunk(0, 0, pl.ds(2 * D, 2 * D))

        def stage(g, m, half):
            c = 3 * g + m
            if half == 0:
                g1, m1 = g, m
            else:
                g1, m1 = jnp.minimum(g + (1 if m == 2 else 0), 3), (m + 1) % 3

            def begin(t, _):
                if t != WAT * half:
                    return
                if half == 1:
                    pl.when(g < 3)(functools.partial(start_chunk, g + 1, m))
                    for at, copy in zip(DMA_AT, other_copies):
                        if at % 3 == m:
                            pl.when(g == at // 3)(copy.start)
                    pl.when(c < 11)(functools.partial(wait_chunk, g1, m1))
                for k in range(4):
                    relayout(g1, m1, 1 - half, k * (D // 8))

            hook = _spread([operands(g1, m1, 1 - half, i0, i0 + 8 if i0 + 8 < D // 8 else None)
                            for i0 in range(0, D // 8, 8)], 45, (WAT + PBEG) * half, 49 * PSUB - PEND)
            rows = P0 // 4 // PSUB
            for sub in range(PSUB):
                zero = g >> (3 + sub + PSUB * (2 * m + half))

                def product(p):
                    if p in _PLAIN:
                        k = _PLAIN.index(p)
                        w = w_s[m][8 * g + 4 * half + k + zero, pl.ds(k * (D // 8), D // 8), :]
                    else:
                        w = forms[half + zero, p]
                    return _dot(_unpack(x49[p + zero, pl.ds(sub * rows // 2, rows // 2), :]),
                                _unpack(w))

                def emit(a, n, v):
                    rings[m * 8 + 4 * half + n][g, pl.ds(a * (P0 // 4) + sub * rows, rows), :] = v

                _products49(product, emit, hooks=[begin, hook], t0=49 * sub)

        @pl.loop(0, 4)
        def _(g):
            for m in range(3):
                for half in range(2):
                    stage(g, m, half)

    pl.run_scoped(
        prologue,
        [pltpu.VMEM((8 * D // 2, DH), u32)] * 3,
        pltpu.VMEM((2, 49, D // 8, DH), u32),
        pltpu.VMEM((49, P0 // 8, C4), u32),
    )
    x_rest[2].start()
    for copy in _late_copies(late_hbm, late_b, sems):
        copy.start()
    for pending in other_copies:
        pending.wait()

    def wrap(r):
        return jnp.where(r >= RING, r - RING, r)

    def stage_tokens(i):
        n = UNROLL * TOK
        tokbuf[...] = _ln(xs[pl.ds(_mult(P0 + n * i, 16), n), :].astype(f32))

    def step(s, carry, tok, resid, first_of_group):
        mem, rp, ra, rw = carry
        ri = lax.broadcasted_iota(jnp.int32, (2 * L, 2 * L), 0)
        ci = lax.broadcasted_iota(jnp.int32, (2 * L, 2 * L), 1)
        same = (ri >= L) == (ci >= L)
        mask = same & ((jnp.where(ri >= L, ri - L, ri) < MEM) | (ri >= ci))
        fill = jnp.where(same, NEG, -jnp.inf)

        lhs = jnp.concatenate([mem, tok], axis=0).astype(bf16)
        rps = [pl.multiple_of(wrap(rp + 8 * i), 8) for i in range(3)]
        ra_ = pl.multiple_of(ra, SEG)
        rw_ = pl.multiple_of(rw, 8)

        col = s & 3
        rb = pl.multiple_of(jnp.maximum((s >> 2) - 1, 0) * (4 * TOK), 8)
        if first_of_group:
            ubuf[...] = _pack(_ln_twice(hbuf[pl.ds(rb, 4 * TOK), :], stats, pl.ds(rb, 4 * TOK)))

        def filler(j):
            r = _dot(_unpack(ubuf[...]), _unpack(w1b[col, :, pl.ds(j * 128, 128)]))
            xg[2 * col + j, pl.ds(HALO + rb, 4 * TOK), :] = _gelu(r)

        mem_qkv = {}
        scores = {}
        o_mem = {}
        total = [None]

        def qkv(h):
            res = []
            for m in range(3):
                r = _dot(lhs, _unpack(w_s[m][h]))
                for i in range(3):
                    ring[m][h][pl.ds(rps[i], 8), :] = r[8 + 8 * i:16 + 8 * i]
                res.append(r[:MEM])
            mem_qkv[h] = res

        def both(h, mem_rows, ring_m):
            return jnp.concatenate(
                [x for k in range(2) for x in (mem_rows[k], ring_m[h + k][pl.ds(ra_, SEG), :])],
                axis=0).astype(bf16)

        def qk(h):
            qm, km, vm = zip(mem_qkv.pop(h), mem_qkv.pop(h + 1))
            sc = lax.dot_general(both(h, qm, q_r), both(h, km, k_r), (((1,), (1,)), ((), ())),
                                 preferred_element_type=f32)
            scores[h] = (sc, vm)

        def pv(h):
            sc, vm = scores.pop(h)
            sc = jnp.where(mask, sc * (DH ** -0.5), fill)
            mx = jnp.max(sc, axis=1, keepdims=True)
            e = jnp.exp(sc - mx)
            den = jnp.sum(e, axis=1, keepdims=True)
            inv = pl.reciprocal(den, approx=True)
            inv = inv * (2.0 - den * inv)
            o = _dot(e.astype(bf16), both(h, vm, v_r)) * inv
            for k in range(2):
                q_r[h + k][pl.ds(ra_, SEG), :] = o[k * L + MEM:(k + 1) * L]
                o_mem[h + k] = o[k * L:k * L + MEM]

        def wo(h):
            lo = jnp.concatenate([o_mem.pop(h), q_r[h][pl.ds(rw_, TOK), :]],
                                 axis=0).astype(bf16)
            r = _dot(lo, _unpack(wo_b[pl.ds(h * DH // 2, DH // 2), :]))
            total[0] = r if total[0] is None else total[0] + r

        slot = {"s": (LAG_QK, qk, 0), "p": (LAG_PV, pv, 0), "a": (0, qkv, 0), "b": (0, qkv, 1),
                "x": (LAG_WO, wo, 0), "y": (LAG_WO, wo, 1)}
        for t in range(H // 2 + LAG_WO + 1):
            for kind in ORDER:
                if kind == "f":
                    for j in range(2):
                        if t == H // 2 + LAG_WO - (FILL_AT if first_of_group else FILL_B)[j]:
                            filler(j)
                    continue
                lag, fn, k = slot[kind]
                if 0 <= t - lag < H // 2:
                    fn(2 * (t - lag) + k)

        a = total[0]
        hbuf[pl.ds(pl.multiple_of(TOK * s, 8), TOK), :] = resid + a[MEM:]
        return a[:MEM], wrap(rp + TOK), wrap(ra + SEG), wrap(rw + TOK)

    def steps(i, carry):
        @pl.when(i == NSEG // UNROLL // 2)
        def _():
            for copy in _late_copies(late_hbm, late_b, sems):
                copy.wait()

        n = UNROLL * TOK
        pl.when(i == (X_LATE - P0) // n - 2)(x_rest[2].wait)
        last = pl.ds(pl.multiple_of(S - P0 + P0 * UNROLL // NSEG * i, 16), P0 * UNROLL // NSEG)
        hbuf[last, :] = xs[last, :].astype(f32)
        toks = tokbuf[...]
        resid = xs[pl.ds(pl.multiple_of(n * i, 16), n), :].astype(f32)
        for k in range(UNROLL):
            rows = slice(k * TOK, (k + 1) * TOK)
            carry = step(i * UNROLL + k, carry, toks[rows], resid[rows], k == 0)
            if k == 0:
                stage_tokens(jnp.minimum(i + 1, NSEG // UNROLL - 1))
        return carry

    stage_tokens(0)
    carry = lax.fori_loop(
        0, NSEG // UNROLL, steps,
        (mem0_ref[...].astype(f32), jnp.int32(P0), jnp.int32(0), jnp.int32(0)))
    zero_ref[0] = carry[1] >> 12


def _block_b(out_hbm, wo_b, hbuf, xg, w1b, late_b, sems, zero_ref, stats, q_rings,
             w3s, w2s, w4s, y49, g49, xbuf, ybuf, res, obuf):
    w2b, w3b, w4b = late_b
    nj = F // FC
    Q = RB // 4

    def out_copy(i, cols=pl.ds(0, D), sem=0):
        rows = pl.ds(_mult(i * RB, RB), RB)
        return pltpu.make_async_copy(obuf.at[i & 1, :, cols], out_hbm.at[rows, cols],
                                     sems.at[SEM_OUT + (i & 1) + sem])

    last_copies = [out_copy(S // RB - 1, pl.ds(k * (D // 2), D // 2), k) for k in range(2)]

    def weight_work(src, dst, row, col, at):
        for grp in range(7):
            def word(k, n):
                return src[pl.ds(_mult(row(k), 8), 8), pl.ds(col(n), 128)]
            for e, v in enumerate(_operands(_RHS, grp, word)):
                dst[at(7 * grp + e)] = v
            yield v

    def w2_work(i, c):
        return weight_work(w2b, w2s, lambda k: k * (D // 8) + i, lambda n: n * C4 + c,
                           lambda p: (p, pl.ds(_mult(i, 8), 8), pl.ds(c, 128)))

    def w3_work(j, i):
        return weight_work(w3b, w3s, lambda k: k * (D // 8) + i, lambda n: j * FC + n * 128,
                           lambda p: (j, p, pl.ds(_mult(i, 8), 8)))

    def w4_work(j, i, c):
        return weight_work(w4b, w4s, lambda k: j * (FC // 2) + k * 64 + i, lambda n: 4 * c + n * 128,
                           lambda p: (p, pl.ds(_mult(j * 64 + i, 8), 8), pl.ds(c, 128)))

    def gather(pieces, p, cols):
        return _unpack(jnp.concatenate(
            [jnp.concatenate([pieces[c, r][p] for r in range(0, Q, 16)], axis=0)
             for c in cols], axis=1))

    def left_work(dst, block, r, c):
        for grp in range(7):
            for e, v in enumerate(_operands(_LHS, grp, block)):
                dst[7 * grp + e, pl.ds(_mult(r // 2, 8), 8), pl.ds(128 * c, 128)] = v
            yield v

    def shift_work(i, r, c):
        def block(a, k):
            r0 = HALO + i * RB + a * Q + r + (-1, 1, -2, 2)[k]
            return [xg[2 * k + c, pl.ds(r0 + z, 8, stride=2), :] for z in range(2)]
        return left_work(g49, block, r, c)

    def y_work(r, c):
        def block(a, k):
            r0 = a * Q + 32 * (r // 32) + (r // 16) % 2
            return [ybuf[2 * k + c, pl.ds(r0 + 2 * z, 8, stride=4), :] for z in range(2)]
        return left_work(y49, block, r, c)

    pieces = [(r, c) for r in range(0, Q, 16) for c in range(2)]

    def mixer_out(i, hooks=()):
        for c in range(0, C4, MW):
            def emit(a, n, v):
                rows, cols = pl.ds(_mult(i * RB + a * Q, Q), Q), pl.ds(n * C4 + c, MW)
                hv = hbuf[rows, cols]
                mean, scale = [jnp.tile(stats[k, rows, :], (1, MW // 128)) for k in range(2)]
                x1 = (hv - mean) * scale + v
                xbuf[pl.ds(a * Q, Q), cols] = x1
                res[i & 1, pl.ds(a * Q, Q), cols] = hv + x1

            _products49(lambda p: _dot(_unpack(g49[p]), _unpack(w2s[p, :, pl.ds(c, MW)])),
                        emit, hooks=hooks, t0=49 * c // MW)

    def norm_x1(r):
        y = _ln(xbuf[pl.ds(r, LN_ROWS), :])
        for k in range(D // 128):
            ybuf[k, pl.ds(r, LN_ROWS), :] = y[:, k * 128:(k + 1) * 128]
        yield

    def post_hooks(zero, t0, t1, t2):
        return [_spread([norm_x1(r) for r in range(0, RB, LN_ROWS)], 1, t0, t1 - LN_GAP, _tie(zero, xbuf)),
                _spread([y_work(r, c) for r, c in pieces], 7, t1, t2, _tie(zero, ybuf))]

    def mlp_block(i, last):
        hidden = {}

        for j in range(nj):
            t = {}
            _products49(lambda p: _dot(_unpack(y49[p]), _unpack(w3s[j, p])),
                        lambda a, n, v: t.__setitem__((a, n), _gelu(v)))
            for r in range(0, Q, 16):
                r0 = 32 * (r // 32) + 8 * ((r // 16) % 2)
                hidden[j, r] = [v for grp in range(7) for v in _operands(
                    _LHS, grp, lambda a, n: [t[a, n][r0 + 16 * z:r0 + 16 * z + 8] for z in range(2)])]

        def down(p, c, j0, j1):
            return _dot(gather(hidden, p, range(j0, j1)),
                        _unpack(w4s[p, pl.ds(64 * j0, 64 * (j1 - j0)), pl.ds(c, 128)]))

        early = {(p, 0): down(p, 0, 0, nj - 1) for p in range(EARLY if last else 0)}
        hooks = []
        if not last:
            mixer_out(i + 1)
            ahead = jnp.minimum(i + 2, S // RB - 1)
            hooks = [_spread([shift_work(ahead, r, c) for r, c in pieces], 7, G_FROM, G_TO,
                             _tie(i >> 3, xg))]
            hooks += post_hooks(i >> 3, 0, Y_FROM, Y_TO)
        for c in range(0, C4, 128):
            def product(p):
                if (p, c) in early:
                    return early.pop((p, c)) + down(p, c, nj - 1, nj)
                return down(p, c, 0, nj)

            def emit(a, n, v):
                obuf[i & 1, pl.ds(a * Q, Q), pl.ds(4 * c + n * 128, 128)] = v.astype(bf16)

            _products49(product, emit,
                        lambda a, n: res[i & 1, pl.ds(a * Q, Q), pl.ds(4 * c + n * 128, 128)],
                        hooks, 49 * c // 128)
            if last:
                last_copies[c // 128].start()

    done = TOK * NSEG
    first = 4 * TOK * (NSEG // 4 - 1)

    @pl.loop(0, H // 8)
    def _(g):
        works = [[w2_work(32 * g + i, c) for i in range(0, 32, 8) for c in range(0, C4, 128)],
                 [shift_work(0, 16 * g, c) for c in range(2)],
                 [w3_work(j, 32 * g + i) for j in range(nj) for i in range(0, 32, 8)],
                 [w4_work(j, 16 * g + i, c) for j in range(nj)
                  for i in range(0, 16, 8) for c in range(0, C4, 128)]]
        per = TK // DH
        calls = P0 // TM * (8 // per) * 8 * TQ - TEND
        ends = [calls * sum(map(len, works[:k])) // sum(map(len, works)) for k in range(5)]
        hooks = [_spread(works[k], 7, ends[k], ends[k + 1], _tie(g >> 2, src))
                 for k, src in enumerate((w2b, xg, w3b, w4b))]
        t = 0
        for r0 in range(done, S, TM):
            rr = r0 % RING
            n = min(TM, RING - rr)
            spans = [(rr, n)] + ([(0, TM - n)] if n < TM else [])
            for k in range(0, 8, per):
                lo = jnp.concatenate(
                    [jnp.concatenate([q_rings[h][g, pl.ds(*span), :] for span in spans], axis=0)
                     for h in range(k, k + per)], axis=1).astype(bf16)
                rows = pl.ds(pl.multiple_of((8 * g + k) * (DH // 2), TK // 2), TK // 2)
                for c in range(0, D, 128):
                    r = _dot(lo, _unpack(wo_b[rows, pl.ds(c, 128)]))
                    for q in range(0, TM, TM // TQ):
                        hbuf[pl.ds(r0 + q, TM // TQ), pl.ds(c, 128)] += r[q:q + TM // TQ]
                        for hook in hooks:
                            hook(t, r[q:q + TM // TQ])
                        t += 1

    zero = zero_ref[0]
    us = {}

    def norm_h(r):
        us[r] = _ln_twice(hbuf[pl.ds(r, UN), :], stats, pl.ds(r, UN))
        yield

    blocks = [(first, done - first)] + [(r0, UM) for r0 in range(done, S, UM)]
    lead = 49 * C4 // MW
    calls = lead + 8 * UQ * len(blocks)
    hooks = [_spread([norm_h(r) for r in range(first, S, UN)], 1, 0, calls - 8 * UQ - ULEAD,
                     _tie(zero, hbuf)),
             _spread([shift_work(1, r, c) for r, c in pieces], 7, lead, calls - 1, _tie(zero, xg))]
    hooks += post_hooks(zero, lead, (lead + calls) // 2, calls - 1)
    mixer_out(0, hooks)
    for b, (r0, n) in enumerate(blocks):
        u = jnp.concatenate([us.pop(r) for r in range(r0, r0 + n, UN)], axis=0).astype(bf16)
        for c in range(D // 128):
            r = _dot(u, _unpack(w1b[c // 2, :, pl.ds(128 * (c % 2), 128)]))
            xg[c, pl.ds(HALO + r0, n), :] = _gelu(r)
            for q in range(UQ):
                for hook in hooks:
                    hook(lead + (8 * b + c) * UQ + q, r[q * n // UQ:(q + 1) * n // UQ])

    @pl.loop(0, S // RB - 1)
    def _(i):
        mlp_block(i, False)
        out_copy(i).start()
        pl.when(i > 0)(lambda: out_copy(i - 1).wait())

    mlp_block(S // RB - 1, True)
    for pending in [out_copy(S // RB - 2)] + last_copies:
        pending.wait()


@jax.jit
def pallas_sequential_preLN__memory_aug_recurrent_mem_tr__mixer_s_mlp__prompt_kernel(
    A_x: jax.Array,
    A_mem0: jax.Array,
    A_Wq: jax.Array,
    A_Wk: jax.Array,
    A_Wv: jax.Array,
    A_Wo: jax.Array,
    A_seg_len: jax.Array,
    B_x: jax.Array,
    B_w1: jax.Array,
    B_w2: jax.Array,
    B_w3: jax.Array,
    B_w4: jax.Array,
):
    del A_seg_len, B_x
    hbm = pl.BlockSpec(memory_space=pl.ANY)
    vmem = pl.BlockSpec(memory_space=pltpu.VMEM)
    scratch = [
        pltpu.VMEM((H * DH // 2, D), u32),
        pltpu.VMEM((S + 8, D), f32),
        pltpu.VMEM((D // 128, S + 2 * HALO + 8, 128), f32),
        pltpu.VMEM((4, D // 2, C4), u32),
        pltpu.VMEM((D // 2 + 8, D), u32),
        pltpu.VMEM((D // 2 + 8, F), u32),
        pltpu.VMEM((F // 2 + 8, D), u32),
        pltpu.SemaphoreType.DMA((NSEM,)),
        pltpu.SMEM((1,), jnp.int32),
        pltpu.VMEM((2, S, 128), f32),
    ] + [pltpu.VMEM((H // 8, RING, DH), f32)] * 8
    out = pl.pallas_call(
        _kernel,
        out_shape=jax.ShapeDtypeStruct((S, D), A_x.dtype),
        in_specs=[hbm, vmem] + [hbm] * 8,
        out_specs=hbm,
        scratch_shapes=scratch,
        compiler_params=pltpu.CompilerParams(
            vmem_limit_bytes=127 * 1024 * 1024,
            flags=[None, {"XLA_TPU_FORCE_LP_LLO_SCHEDULER": True}, {"XLA_TPU_EVENLY_DISTRIBUTE_CRITICAL_NODES": True}][FLAG]),
    )(A_x.reshape(S, D), A_mem0.reshape(MEM, D),
      A_Wq, A_Wk, A_Wv,
      A_Wo.reshape(H * DH, D), B_w1, B_w2, B_w3, B_w4)
    return out.reshape(A_x.shape)
```

```python
import functools

import jax
import jax.numpy as jnp
from jax import lax
import jax.experimental.pallas as pl
import jax.experimental.pallas.tpu as pltpu

S = 2048
D = 1024
H = 32
DH = 128
MEM = 8
SEG = 32
F = 3584
NSEG = S // SEG
L = MEM + SEG
TOK = 24
P0 = S - TOK * NSEG
RING = 576
C4 = D // 4
HALO = 8
RB = 256
FC = 512
EPS = 1e-5
NEG = -1000000000.0

X_LATE = 704

PSUB = 2
WAT = 1
PEND = 2
RG = 2
RAT = (0, 1, 4, 5)
DMA_AT = (2, 4, 6, 9, 8, 9, 9)

LAG_QK = 2
LAG_PV = 4
LAG_WO = 5
ORDER = "pbsafxy"
FILL_AT = (4, 0)
FILL_B = (4, 4)
FILL_N = 1
UNROLL = 2

TM = 128
TK = 512
TQ = 8
TEND = 8
UM = 64
ULEAD = 120
LN_ROWS = 8
LN_GAP = 2
Y_FROM = 38
G_FROM = 68
G_TO = 97
EARLY = 16

bf16 = jnp.bfloat16
f32 = jnp.float32
u32 = jnp.uint32

SEM_X, SEM_XR, SEM_WO, SEM_W1, SEM_W2, SEM_OUT, SEM_W0, SEM_W = 0, 4, 7, 11, 15, 18, 21, 22
NSEM = SEM_W + 12


def _mult(i, n):
    return i if isinstance(i, int) else pl.multiple_of(i, n)


def _ln(x):
    m = jnp.mean(x, axis=-1, keepdims=True)
    d = x - m
    v = jnp.mean(d * d, axis=-1, keepdims=True)
    return d * lax.rsqrt(v + EPS)


def _ln_twice(x, stats, rows):
    m = jnp.mean(x, axis=-1, keepdims=True)
    d = x - m
    scale = lax.rsqrt(jnp.mean(d * d, axis=-1, keepdims=True) + EPS)
    for k, v in enumerate((m, scale)):
        stats[k, rows, :] = jnp.broadcast_to(v, (x.shape[0], 128))
    return _ln(d * scale)


def _gelu(x):
    return jax.nn.gelu(x, approximate=True)


def _pack(x):
    return pltpu.bitcast(x.astype(bf16), u32)


def _unpack(x):
    return pltpu.bitcast(x, bf16)


def _pack2(even, odd):
    return pltpu.pack_elementwise([even, odd], packed_dtype=bf16)


def _half(w, i):
    return pltpu.unpack_elementwise(w, index=i, packed_dtype=bf16, unpacked_dtype=f32)


def _dot(a, b):
    return jnp.dot(a, b, preferred_element_type=f32)


_LHS = ((2, -1, 0), (2, 1, 3), (3, 0, None), (0, 1, 3), (0, 0, None), (0, 1, 1), (1, -1, 3))
_RHS = ((0, 1, 1), (0, 0, None), (2, -1, 0), (0, 1, 3), (1, -1, 3), (3, 0, None), (2, 1, 3))
_USES = (((3, 1),), ((2, 1), (3, -1)), ((2, 1), (0, 1)), ((0, 1), (3, 1)),
         ((3, 1), (1, 1)), ((1, 1), (0, -1)), ((0, 1),))
_LAST = (6, 5, 2, 4)
_PLAIN = (8, 12, 36, 40)


def _operands(table, g, block):
    def halves(x):
        return x if isinstance(x, (list, tuple)) else [_half(x, 0), _half(x, 1)]

    def comb(x, sign, y):
        return [a + b if sign > 0 else a - b for a, b in zip(halves(x), halves(y))]

    i, sign, j = table[g]
    inner = []
    for r in range(2):
        for c in range(2):
            x = block(2 * (i // 2) + r, 2 * (i % 2) + c)
            inner.append(comb(x, sign, block(2 * (j // 2) + r, 2 * (j % 2) + c)) if sign else x)
    out = []
    for i, sign, j in table:
        x = comb(inner[i], sign, inner[j]) if sign else inner[i]
        out.append(_pack2(*x) if isinstance(x, (list, tuple)) else x)
    return out


def _left7(u):
    r, c = u.shape[0] // 2, u.shape[1] // 2
    x = [u[:r, :c], u[:r, c:], u[r:, :c], u[r:, c:]]
    return [x[i] if not sign else x[i] + x[j] if sign > 0 else x[i] - x[j] for i, sign, j in _LHS]


def _products7(product, emit):
    total = [None] * 4
    for e in range(7):
        m = product(e)
        for q, sign in _USES[e]:
            total[q] = m if total[q] is None else total[q] + m if sign > 0 else total[q] - m
            if e == _LAST[q]:
                emit(q, total[q])
        yield m


def _spread(works, steps, first, last, before=None):
    work = (v for w in works for v in w)
    total, n = steps * len(works), last - first

    def hook(t, result):
        if first <= t < last:
            count = (t + 1 - first) * total // n - (t - first) * total // n
            for k in range(count):
                if before is not None:
                    r = k * result.shape[0] // (8 * count) * 8
                    before(result[r:r + 8, :128])
                next(work)
    return hook


def _tie(zero, ref):
    def write(v):
        rows = pl.ds(pl.multiple_of(ref.shape[-2] - 8 + 8 * zero, 8), 8)
        ref[(zero,) * (len(ref.shape) - 2) + (rows, pl.ds(0, 128))] = pltpu.bitcast(v, ref.dtype)
    return write


def _products49(product, emit, start=None, hooks=(), t0=0):
    total = {}
    for g in range(7):
        def emit_inner(q, v):
            for o, sign in _USES[g]:
                rc = (2 * (o // 2) + q // 2, 2 * (o % 2) + q % 2)
                if rc not in total:
                    total[rc] = v if start is None else start(*rc) + v
                else:
                    total[rc] = total[rc] + v if sign > 0 else total[rc] - v
                if g == _LAST[o]:
                    emit(*rc, total.pop(rc))

        for e, m in enumerate(_products7(lambda e: product(7 * g + e), emit_inner)):
            for hook in hooks:
                hook(t0 + 7 * g + e, m)


def _kernel(x_hbm, mem0_ref, wq_hbm, wk_hbm, wv_hbm, wo_hbm, w1_hbm, w2_hbm,
            w3_hbm, w4_hbm, out_hbm,
            wo_b, hbuf, xg, w1s, w2b, w3b, w4b, sems, zero_ref, stats, *q_rings):
    pl.run_scoped(
        functools.partial(_block_a, x_hbm, mem0_ref, (wq_hbm, wk_hbm, wv_hbm), wo_hbm,
                          w1_hbm, (w2_hbm, w3_hbm, w4_hbm), wo_b, hbuf, xg, w1s,
                          (w2b, w3b, w4b), sems, zero_ref, stats, q_rings),
        [pltpu.VMEM((H, D // 2, DH), u32)] * 3,
        [pltpu.VMEM((H // 8, RING, DH), f32)] * 16,
        pltpu.VMEM((7, TOK, D // 2), u32),
        pltpu.VMEM((D // 2, D), u32),
        pltpu.VMEM((S, D), bf16),
        pltpu.VMEM((UNROLL * TOK, D), f32),
    )
    pl.run_scoped(
        functools.partial(_block_b, out_hbm, wo_b, hbuf, xg,
                          w1s, (w2b, w3b, w4b), sems, zero_ref, stats, q_rings),
        pltpu.VMEM((F // FC, 49, D // 8, 128), u32),
        pltpu.VMEM((49, D // 8, C4), u32),
        pltpu.VMEM((49, F // 8, C4), u32),
        pltpu.VMEM((49, RB // 8, C4), u32),
        pltpu.VMEM((49, RB // 8, C4), u32),
        pltpu.VMEM((RB + 8, D), f32),
        pltpu.VMEM((D // 128, RB + 8, 128), f32),
        pltpu.VMEM((2, RB, D), f32),
        pltpu.VMEM((2, RB, D), bf16),
    )


def _late_copies(w_hbm, w_b, sems):
    return [pltpu.make_async_copy(src.bitcast(u32), dst.at[pl.ds(0, dst.shape[0] - 8)],
                                  sems.at[SEM_W2 + i])
            for i, (src, dst) in enumerate(zip(w_hbm, w_b))]


def _block_a(x_hbm, mem0_ref, w_hbm, wo_hbm, w1_hbm, late_hbm, wo_b, hbuf, xg, w1s,
             late_b, sems, zero_ref, stats, q_rings, w_s, kv_rings, ubuf, w1b, xs, tokbuf):
    rings = list(q_rings) + list(kv_rings)
    ring = [[rings[m * 8 + h % 8].at[h // 8] for h in range(H)] for m in range(3)]
    q_r, k_r, v_r = ring

    def wo_copy(i):
        rows = pl.ds(i * 512, 512)
        return pltpu.make_async_copy(wo_hbm.bitcast(u32).at[rows], wo_b.at[rows],
                                     sems.at[SEM_WO + i])

    w1_copy = pltpu.make_async_copy(w1_hbm.bitcast(u32), w1b, sems.at[SEM_W1])

    x_rest = [pltpu.make_async_copy(x_hbm.at[pl.ds(r0, r1 - r0)], xs.at[pl.ds(r0, r1 - r0)],
                                    sems.at[SEM_XR + i])
              for i, (r0, r1) in enumerate(((P0, X_LATE), (S - P0, S), (X_LATE, S - P0)))]
    other_copies = [wo_copy(i) for i in range(4)] + [w1_copy] + x_rest[:2]

    def prologue(stg, forms, x49):
        def start_chunk(g, m, pairs=range(4), sem=None):
            for pair in pairs:
                pltpu.make_async_copy(
                    w_hbm[m].bitcast(u32).at[:, 4 * g + pair, :], stg[m].at[pl.ds(pair * D, D)],
                    sems.at[SEM_W + 3 * g + m if sem is None else sem]).start()

        def wait_chunk(g, m, rows=pl.ds(0, 4 * D), sem=None):
            pltpu.make_async_copy(stg[m].at[rows], stg[m].at[rows],
                                  sems.at[SEM_W + 3 * g + m if sem is None else sem]).wait()

        def relayout(g, m, half, i):
            for a in range(2):
                ev, od = [stg[m][pl.ds((2 * half + a) * D + 2 * i + par, 8, stride=2), :]
                          for par in range(2)]
                for z in range(2):
                    w_s[m][8 * g + 4 * half + 2 * a + z, pl.ds(i, 8), :] = _pack2(
                        _half(ev, z), _half(od, z))

        def operands(g, m, half, i0, ahead):
            for grp in range(7):
                def word(k, n):
                    return w_s[m][8 * g + 4 * half + n + (g >> (4 + grp // RG)),
                                  pl.ds(k * (D // 8) + i0, 8), :]
                for e, v in enumerate(_operands(_RHS, grp, word)):
                    if 7 * grp + e not in _PLAIN:
                        forms[half + (g >> 2), 7 * grp + e, pl.ds(i0, 8), :] = v
                        yield
                if ahead is not None and grp in RAT:
                    relayout(g, m, half, RAT.index(grp) * (D // 8) + ahead)

        def x_copy(i):
            rows = pl.ds(_mult(i * 128, 128), 128)
            return pltpu.make_async_copy(x_hbm.at[rows], xs.at[rows], sems.at[SEM_X + i])

        start_chunk(0, 0, range(2), SEM_W0)
        for i in range(P0 // 128):
            x_copy(i).start()
        start_chunk(0, 0, range(2, 4))
        for m in range(1, 3):
            start_chunk(0, m)
        zero = jnp.zeros((HALO, 128), f32)
        for c in range(D // 128):
            xg[c, pl.ds(0, HALO), :] = zero
            xg[c, pl.ds(HALO + S, HALO), :] = zero
        hbuf[pl.ds(0, 4 * TOK), :] = jnp.zeros((4 * TOK, D), f32)
        wait_chunk(0, 0, pl.ds(0, 2 * D), SEM_W0)

        @pl.loop(0, D // 64)
        def _(i):
            for k in range(4):
                relayout(0, 0, 0, pl.multiple_of(k * (D // 8) + 8 * i, 8))
            for _ in operands(0, 0, 0, pl.multiple_of(8 * i, 8), None):
                pass

        @pl.loop(0, P0 // 128)
        def _(i):
            x_copy(i).wait()
            r0 = pl.multiple_of(i * 128, 128)
            xn = _ln(xs[pl.ds(r0, 128), :].astype(f32))
            for c in range(D // 128):
                xg[c, pl.ds(HALO + r0, 128), :] = xn[:, c * 128:(c + 1) * 128]

        @pl.loop(0, P0 // 64)
        def _(i):
            for c in range(2):
                def block(a, k):
                    return [xg[2 * k + c, pl.ds(HALO + a * (P0 // 4) + 16 * i + z, 8, stride=2), :]
                            for z in range(2)]
                for grp in range(7):
                    for e, v in enumerate(_operands(_LHS, grp, block)):
                        x49[7 * grp + e, pl.ds(pl.multiple_of(8 * i, 8), 8), pl.ds(128 * c, 128)] = v

        wait_chunk(0, 0, pl.ds(2 * D, 2 * D))

        def stage(g, m, half):
            c = 3 * g + m
            if half == 0:
                g1, m1 = g, m
            else:
                g1, m1 = jnp.minimum(g + (1 if m == 2 else 0), 3), (m + 1) % 3

            def begin(t, _):
                if t != WAT * half:
                    return
                if half == 1:
                    pl.when(g < 3)(functools.partial(start_chunk, g + 1, m))
                    for at, copy in zip(DMA_AT, other_copies):
                        if at % 3 == m:
                            pl.when(g == at // 3)(copy.start)
                    pl.when(c < 11)(functools.partial(wait_chunk, g1, m1))
                for k in range(4):
                    relayout(g1, m1, 1 - half, k * (D // 8))

            hook = _spread([operands(g1, m1, 1 - half, i0, i0 + 8 if i0 + 8 < D // 8 else None)
                            for i0 in range(0, D // 8, 8)], 45, (WAT + 1) * half, 49 * PSUB - PEND)
            rows = P0 // 4 // PSUB
            for sub in range(PSUB):
                zero = g >> (3 + sub + PSUB * (2 * m + half))

                def product(p):
                    if p in _PLAIN:
                        k = _PLAIN.index(p)
                        w = w_s[m][8 * g + 4 * half + k + zero, pl.ds(k * (D // 8), D // 8), :]
                    else:
                        w = forms[half + zero, p]
                    return _dot(_unpack(x49[p + zero, pl.ds(sub * rows // 2, rows // 2), :]),
                                _unpack(w))

                def emit(a, n, v):
                    rings[m * 8 + 4 * half + n][g, pl.ds(a * (P0 // 4) + sub * rows, rows), :] = v

                _products49(product, emit, hooks=[begin, hook], t0=49 * sub)

        @pl.loop(0, 4)
        def _(g):
            for m in range(3):
                for half in range(2):
                    stage(g, m, half)

    pl.run_scoped(
        prologue,
        [pltpu.VMEM((4 * D + 8, DH), u32)] * 3,
        pltpu.VMEM((2, 49, D // 8, DH), u32),
        pltpu.VMEM((49, P0 // 8, C4), u32),
    )
    x_rest[2].start()
    for copy in _late_copies(late_hbm, late_b, sems):
        copy.start()
    for pending in other_copies:
        pending.wait()

    @pl.loop(0, D // 32)
    def _(i):
        for c in range(4):
            x = [w1b[pl.ds(pl.multiple_of(k * (D // 4) + 8 * i, 8), 8),
                     pl.ds(n * (D // 2) + 128 * c, 128)] for k in range(2) for n in range(2)]
            for e, (a, sign, b) in enumerate(_RHS):
                halves = [(_half(x[a], z), _half(x[b], z)) for z in range(2)] if sign else None
                w1s[c, e, pl.ds(pl.multiple_of(8 * i, 8), 8), :] = x[a] if not sign else _pack2(
                    *[u + v if sign > 0 else u - v for u, v in halves])

    def wrap(r):
        return jnp.where(r >= RING, r - RING, r)

    def stage_tokens(i):
        n = UNROLL * TOK
        tokbuf[...] = _ln(xs[pl.ds(_mult(P0 + n * i, 16), n), :].astype(f32))

    def step(s, carry, tok, resid, first_of_group):
        mem, rp, ra, rw = carry
        ri = lax.broadcasted_iota(jnp.int32, (2 * L, 2 * L), 0)
        ci = lax.broadcasted_iota(jnp.int32, (2 * L, 2 * L), 1)
        same = (ri >= L) == (ci >= L)
        mask = same & ((jnp.where(ri >= L, ri - L, ri) < MEM) | (ri >= ci))
        fill = jnp.where(same, NEG, -jnp.inf)

        lhs = jnp.concatenate([mem, tok], axis=0).astype(bf16)
        rps = [pl.multiple_of(wrap(rp + 8 * i), 8) for i in range(3)]
        ra_ = pl.multiple_of(ra, SEG)
        rw_ = pl.multiple_of(rw, 8)

        col = s & 3
        rb = pl.multiple_of(jnp.maximum((s >> 2) - 1, 0) * (4 * TOK), 8)
        if first_of_group:
            u = _ln_twice(hbuf[pl.ds(rb, 4 * TOK), :], stats, pl.ds(rb, 4 * TOK))
            for e, v in enumerate(_left7(u)):
                ubuf[e] = _pack(v)

        def emit(q, v):
            xg[4 * (q % 2) + col, pl.ds(HALO + rb + 2 * TOK * (q // 2), 2 * TOK), :] = _gelu(v)

        fill_work = _products7(lambda e: _dot(_unpack(ubuf[e]), _unpack(w1s[col, e])), emit)

        def filler(j):
            for _ in range((FILL_N, 7 - FILL_N)[j]):
                next(fill_work)

        mem_qkv = {}
        scores = {}
        o_mem = {}
        total = [None]

        def qkv(h):
            res = []
            for m in range(3):
                r = _dot(lhs, _unpack(w_s[m][h]))
                for i in range(3):
                    ring[m][h][pl.ds(rps[i], 8), :] = r[8 + 8 * i:16 + 8 * i]
                res.append(r[:MEM])
            mem_qkv[h] = res

        def both(h, mem_rows, ring_m):
            return jnp.concatenate(
                [x for k in range(2) for x in (mem_rows[k], ring_m[h + k][pl.ds(ra_, SEG), :])],
                axis=0).astype(bf16)

        def qk(h):
            qm, km, vm = zip(mem_qkv.pop(h), mem_qkv.pop(h + 1))
            sc = lax.dot_general(both(h, qm, q_r), both(h, km, k_r), (((1,), (1,)), ((), ())),
                                 preferred_element_type=f32)
            scores[h] = (sc, vm)

        def pv(h):
            sc, vm = scores.pop(h)
            sc = jnp.where(mask, sc * (DH ** -0.5), fill)
            mx = jnp.max(sc, axis=1, keepdims=True)
            e = jnp.exp(sc - mx)
            den = jnp.sum(e, axis=1, keepdims=True)
            inv = pl.reciprocal(den, approx=True)
            inv = inv * (2.0 - den * inv)
            o = _dot(e.astype(bf16), both(h, vm, v_r)) * inv
            for k in range(2):
                q_r[h + k][pl.ds(ra_, SEG), :] = o[k * L + MEM:(k + 1) * L]
                o_mem[h + k] = o[k * L:k * L + MEM]

        def wo(h):
            lo = jnp.concatenate([o_mem.pop(h), q_r[h][pl.ds(rw_, TOK), :]],
                                 axis=0).astype(bf16)
            r = _dot(lo, _unpack(wo_b[pl.ds(h * DH // 2, DH // 2), :]))
            total[0] = r if total[0] is None else total[0] + r

        slot = {"s": (LAG_QK, qk, 0), "p": (LAG_PV, pv, 0), "a": (0, qkv, 0), "b": (0, qkv, 1),
                "x": (LAG_WO, wo, 0), "y": (LAG_WO, wo, 1)}
        for t in range(H // 2 + LAG_WO + 1):
            for kind in ORDER:
                if kind == "f":
                    for j in range(2):
                        if t == H // 2 + LAG_WO - (FILL_AT if first_of_group else FILL_B)[j]:
                            filler(j)
                    continue
                lag, fn, k = slot[kind]
                if 0 <= t - lag < H // 2:
                    fn(2 * (t - lag) + k)

        a = total[0]
        hbuf[pl.ds(pl.multiple_of(TOK * s, 8), TOK), :] = resid + a[MEM:]
        return a[:MEM], wrap(rp + TOK), wrap(ra + SEG), wrap(rw + TOK)

    def steps(i, carry):
        @pl.when(i == NSEG // UNROLL // 2)
        def _():
            for copy in _late_copies(late_hbm, late_b, sems):
                copy.wait()

        n = UNROLL * TOK
        pl.when(i == (X_LATE - P0) // n - 2)(x_rest[2].wait)
        last = pl.ds(pl.multiple_of(S - P0 + P0 * UNROLL // NSEG * i, 16), P0 * UNROLL // NSEG)
        hbuf[last, :] = xs[last, :].astype(f32)
        toks = tokbuf[...]
        resid = xs[pl.ds(pl.multiple_of(n * i, 16), n), :].astype(f32)
        for k in range(UNROLL):
            rows = slice(k * TOK, (k + 1) * TOK)
            carry = step(i * UNROLL + k, carry, toks[rows], resid[rows], k == 0)
            if k == 0:
                stage_tokens(jnp.minimum(i + 1, NSEG // UNROLL - 1))
        return carry

    stage_tokens(0)
    carry = lax.fori_loop(
        0, NSEG // UNROLL, steps,
        (mem0_ref[...].astype(f32), jnp.int32(P0), jnp.int32(0), jnp.int32(0)))
    zero_ref[0] = carry[1] >> 12


def _block_b(out_hbm, wo_b, hbuf, xg, w1s, late_b, sems, zero_ref, stats, q_rings,
             w3s, w2s, w4s, y49, g49, xbuf, ybuf, res, obuf):
    w2b, w3b, w4b = late_b
    nj = F // FC
    Q = RB // 4

    def out_copy(i, cols=pl.ds(0, D), sem=0):
        rows = pl.ds(_mult(i * RB, RB), RB)
        return pltpu.make_async_copy(obuf.at[i & 1, :, cols], out_hbm.at[rows, cols],
                                     sems.at[SEM_OUT + (i & 1) + sem])

    last_copies = [out_copy(S // RB - 1, pl.ds(k * (D // 2), D // 2), k) for k in range(2)]

    def weight_work(src, dst, row, col, at):
        for grp in range(7):
            def word(k, n):
                return src[pl.ds(_mult(row(k), 8), 8), pl.ds(col(n), 128)]
            for e, v in enumerate(_operands(_RHS, grp, word)):
                dst[at(7 * grp + e)] = v
            yield

    def w2_work(i, c):
        return weight_work(w2b, w2s, lambda k: k * (D // 8) + i, lambda n: n * C4 + c,
                           lambda p: (p, pl.ds(_mult(i, 8), 8), pl.ds(c, 128)))

    def w3_work(j, i):
        return weight_work(w3b, w3s, lambda k: k * (D // 8) + i, lambda n: j * FC + n * 128,
                           lambda p: (j, p, pl.ds(_mult(i, 8), 8)))

    def w4_work(j, i, c):
        return weight_work(w4b, w4s, lambda k: j * (FC // 2) + k * 64 + i, lambda n: 4 * c + n * 128,
                           lambda p: (p, pl.ds(_mult(j * 64 + i, 8), 8), pl.ds(c, 128)))

    def gather(pieces, p, cols):
        return _unpack(jnp.concatenate(
            [jnp.concatenate([pieces[c, r][p] for r in range(0, Q, 16)], axis=0)
             for c in cols], axis=1))

    def left_work(dst, block, r, c):
        for grp in range(7):
            for e, v in enumerate(_operands(_LHS, grp, block)):
                dst[7 * grp + e, pl.ds(_mult(r // 2, 8), 8), pl.ds(128 * c, 128)] = v
            yield

    def shift_work(i, r, c):
        def block(a, k):
            r0 = HALO + i * RB + a * Q + r + (-1, 1, -2, 2)[k]
            return [xg[2 * k + c, pl.ds(r0 + z, 8, stride=2), :] for z in range(2)]
        return left_work(g49, block, r, c)

    def y_work(r, c):
        def block(a, k):
            r0 = a * Q + 32 * (r // 32) + (r // 16) % 2
            return [ybuf[2 * k + c, pl.ds(r0 + 2 * z, 8, stride=4), :] for z in range(2)]
        return left_work(y49, block, r, c)

    pieces = [(r, c) for r in range(0, Q, 16) for c in range(2)]

    def mixer_out(i, hooks=()):
        for c in range(0, C4, 128):
            def emit(a, n, v):
                rows, cols = pl.ds(_mult(i * RB + a * Q, Q), Q), pl.ds(n * C4 + c, 128)
                hv = hbuf[rows, cols]
                x1 = (hv - stats[0, rows, :]) * stats[1, rows, :] + v
                xbuf[pl.ds(a * Q, Q), cols] = x1
                res[i & 1, pl.ds(a * Q, Q), cols] = hv + x1

            _products49(lambda p: _dot(_unpack(g49[p]), _unpack(w2s[p, :, pl.ds(c, 128)])),
                        emit, hooks=hooks, t0=49 * c // 128)

    def norm_x1(r):
        y = _ln(xbuf[pl.ds(r, LN_ROWS), :])
        for k in range(D // 128):
            ybuf[k, pl.ds(r, LN_ROWS), :] = y[:, k * 128:(k + 1) * 128]
        yield

    def post_hooks(zero, t0, t1, t2):
        return [_spread([norm_x1(r) for r in range(0, RB, LN_ROWS)], 1, t0, t1 - LN_GAP, _tie(zero, xbuf)),
                _spread([y_work(r, c) for r, c in pieces], 7, t1, t2, _tie(zero, ybuf))]

    def mlp_block(i, last):
        hidden = {}

        for j in range(nj):
            t = {}
            _products49(lambda p: _dot(_unpack(y49[p]), _unpack(w3s[j, p])),
                        lambda a, n, v: t.__setitem__((a, n), _gelu(v)))
            for r in range(0, Q, 16):
                r0 = 32 * (r // 32) + 8 * ((r // 16) % 2)
                hidden[j, r] = [v for grp in range(7) for v in _operands(
                    _LHS, grp, lambda a, n: [t[a, n][r0 + 16 * z:r0 + 16 * z + 8] for z in range(2)])]

        def down(p, c, j0, j1):
            return _dot(gather(hidden, p, range(j0, j1)),
                        _unpack(w4s[p, pl.ds(64 * j0, 64 * (j1 - j0)), pl.ds(c, 128)]))

        early = {(p, 0): down(p, 0, 0, nj - 1) for p in range(EARLY if last else 0)}
        hooks = []
        if not last:
            mixer_out(i + 1)
            ahead = jnp.minimum(i + 2, S // RB - 1)
            hooks = [_spread([shift_work(ahead, r, c) for r, c in pieces], 7, G_FROM, G_TO,
                             _tie(i >> 3, xg))]
            hooks += post_hooks(i >> 3, 0, Y_FROM, G_FROM)
        for c in range(0, C4, 128):
            def product(p):
                if (p, c) in early:
                    return early.pop((p, c)) + down(p, c, nj - 1, nj)
                return down(p, c, 0, nj)

            def emit(a, n, v):
                obuf[i & 1, pl.ds(a * Q, Q), pl.ds(4 * c + n * 128, 128)] = v.astype(bf16)

            _products49(product, emit,
                        lambda a, n: res[i & 1, pl.ds(a * Q, Q), pl.ds(4 * c + n * 128, 128)],
                        hooks, 49 * c // 128)
            if last:
                last_copies[c // 128].start()

    done = TOK * NSEG
    first = 4 * TOK * (NSEG // 4 - 1)

    @pl.loop(0, H // 8)
    def _(g):
        works = [[w2_work(32 * g + i, c) for i in range(0, 32, 8) for c in range(0, C4, 128)],
                 [shift_work(0, 16 * g, c) for c in range(2)],
                 [w3_work(j, 32 * g + i) for j in range(nj) for i in range(0, 32, 8)],
                 [w4_work(j, 16 * g + i, c) for j in range(nj)
                  for i in range(0, 16, 8) for c in range(0, C4, 128)]]
        per = TK // DH
        calls = P0 // TM * (8 // per) * 8 * TQ - TEND
        ends = [calls * sum(map(len, works[:k])) // sum(map(len, works)) for k in range(5)]
        hooks = [_spread(works[k], 7, ends[k], ends[k + 1], _tie(g >> 2, src))
                 for k, src in enumerate((w2b, xg, w3b, w4b))]
        t = 0
        for r0 in range(done, S, TM):
            rr = r0 % RING
            n = min(TM, RING - rr)
            spans = [(rr, n)] + ([(0, TM - n)] if n < TM else [])
            for k in range(0, 8, per):
                lo = jnp.concatenate(
                    [jnp.concatenate([q_rings[h][g, pl.ds(*span), :] for span in spans], axis=0)
                     for h in range(k, k + per)], axis=1).astype(bf16)
                rows = pl.ds(pl.multiple_of((8 * g + k) * (DH // 2), TK // 2), TK // 2)
                for c in range(0, D, 128):
                    r = _dot(lo, _unpack(wo_b[rows, pl.ds(c, 128)]))
                    for q in range(0, TM, TM // TQ):
                        hbuf[pl.ds(r0 + q, TM // TQ), pl.ds(c, 128)] += r[q:q + TM // TQ]
                        for hook in hooks:
                            hook(t, r[q:q + TM // TQ])
                        t += 1

    zero = zero_ref[0]
    us = {}

    def norm_h(r):
        us[r] = _ln_twice(hbuf[pl.ds(r, LN_ROWS), :], stats, pl.ds(r, LN_ROWS))
        yield

    blocks = [(first, done - first)] + [(r0, UM) for r0 in range(done, S, UM)]
    lead = 2 * 49
    calls = lead + 28 * len(blocks)
    hooks = [_spread([norm_h(r) for r in range(first, S, LN_ROWS)], 1, 0, calls - 28 - ULEAD,
                     _tie(zero, hbuf)),
             _spread([shift_work(1, r, c) for r, c in pieces], 7, lead, calls - 1, _tie(zero, xg))]
    hooks += post_hooks(zero, lead, (lead + calls) // 2, calls - 1)
    mixer_out(0, hooks)
    for b, (r0, n) in enumerate(blocks):
        left = _left7(jnp.concatenate([us.pop(r) for r in range(r0, r0 + n, LN_ROWS)], axis=0))
        for c in range(4):
            def emit(q, v):
                xg[4 * (q % 2) + c, pl.ds(HALO + r0 + n // 2 * (q // 2), n // 2), :] = _gelu(v)

            for e, m in enumerate(_products7(
                    lambda e: _dot(left[e].astype(bf16), _unpack(w1s[c, e])), emit)):
                for hook in hooks:
                    hook(lead + 28 * b + 7 * c + e, m)

    @pl.loop(0, S // RB - 1)
    def _(i):
        mlp_block(i, False)
        out_copy(i).start()
        pl.when(i > 0)(lambda: out_copy(i - 1).wait())

    mlp_block(S // RB - 1, True)
    for pending in [out_copy(S // RB - 2)] + last_copies:
        pending.wait()


@jax.jit
def pallas_sequential_preLN__memory_aug_recurrent_mem_tr__mixer_s_mlp__prompt_kernel(
    A_x: jax.Array,
    A_mem0: jax.Array,
    A_Wq: jax.Array,
    A_Wk: jax.Array,
    A_Wv: jax.Array,
    A_Wo: jax.Array,
    A_seg_len: jax.Array,
    B_x: jax.Array,
    B_w1: jax.Array,
    B_w2: jax.Array,
    B_w3: jax.Array,
    B_w4: jax.Array,
):
    del A_seg_len, B_x
    hbm = pl.BlockSpec(memory_space=pl.ANY)
    vmem = pl.BlockSpec(memory_space=pltpu.VMEM)
    scratch = [
        pltpu.VMEM((H * DH // 2, D), u32),
        pltpu.VMEM((S + 8, D), f32),
        pltpu.VMEM((D // 128, S + 2 * HALO + 8, 128), f32),
        pltpu.VMEM((4, 7, D // 4, 128), u32),
        pltpu.VMEM((D // 2 + 8, D), u32),
        pltpu.VMEM((D // 2 + 8, F), u32),
        pltpu.VMEM((F // 2 + 8, D), u32),
        pltpu.SemaphoreType.DMA((NSEM,)),
        pltpu.SMEM((1,), jnp.int32),
        pltpu.VMEM((2, S, 128), f32),
    ] + [pltpu.VMEM((H // 8, RING, DH), f32)] * 8
    out = pl.pallas_call(
        _kernel,
        out_shape=jax.ShapeDtypeStruct((S, D), A_x.dtype),
        in_specs=[hbm, vmem] + [hbm] * 8,
        out_specs=hbm,
        scratch_shapes=scratch,
        compiler_params=pltpu.CompilerParams(vmem_limit_bytes=255 * 512 * 1024),
    )(A_x.reshape(S, D), A_mem0.reshape(MEM, D),
      A_Wq, A_Wk, A_Wv,
      A_Wo.reshape(H * DH, D), B_w1, B_w2, B_w3, B_w4)
    return out.reshape(A_x.shape)
```

```python
import functools

import jax
import jax.numpy as jnp
from jax import lax
import jax.experimental.pallas as pl
import jax.experimental.pallas.tpu as pltpu

S = 2048
D = 1024
H = 32
DH = 128
MEM = 8
SEG = 32
F = 3584
NSEG = S // SEG
L = MEM + SEG
TOK = 24
P0 = S - TOK * NSEG
RING = 576
C4 = D // 4
HALO = 8
RB = 256
FC = 512
EPS = 1e-5
NEG = -1000000000.0

X_LATE = 704

PSUB = 2
WAT = 1
PEND = 2
RG = 2
RAT = (0, 1, 4, 5)
DMA_AT = (2, 4, 6, 9, 8, 9, 9)

LAG_QK = 2
LAG_PV = 4
LAG_WO = 5
ORDER = "pbsafxy"
FILL_AT = (4, 0)
FILL_B = (4, 4)
FILL_N = 1
UNROLL = 2

TM = 128
TK = 512
TQ = 8
TEND = 8
UM = 64
ULEAD = 120
LN_ROWS = 8
LN_GAP = 1
Y_FROM = 42
G_FROM = 72
G_TO = 97
H_FROM = 4
H_TO = 48
EARLY = 16

bf16 = jnp.bfloat16
f32 = jnp.float32
u32 = jnp.uint32

SEM_X, SEM_XR, SEM_WO, SEM_W1, SEM_W2, SEM_OUT, SEM_W0, SEM_W = 0, 4, 7, 11, 15, 18, 21, 22
NSEM = SEM_W + 12


def _mult(i, n):
    return i if isinstance(i, int) else pl.multiple_of(i, n)


def _ln(x):
    m = jnp.mean(x, axis=-1, keepdims=True)
    d = x - m
    v = jnp.mean(d * d, axis=-1, keepdims=True)
    return d * lax.rsqrt(v + EPS)


def _ln_twice(x, stats, rows):
    m = jnp.mean(x, axis=-1, keepdims=True)
    d = x - m
    scale = lax.rsqrt(jnp.mean(d * d, axis=-1, keepdims=True) + EPS)
    for k, v in enumerate((m, scale)):
        stats[k, rows, :] = jnp.broadcast_to(v, (x.shape[0], 128))
    return _ln(d * scale)


def _gelu(x):
    return jax.nn.gelu(x, approximate=True)


def _pack(x):
    return pltpu.bitcast(x.astype(bf16), u32)


def _unpack(x):
    return pltpu.bitcast(x, bf16)


def _pack2(even, odd):
    return pltpu.pack_elementwise([even, odd], packed_dtype=bf16)


def _half(w, i):
    return pltpu.unpack_elementwise(w, index=i, packed_dtype=bf16, unpacked_dtype=f32)


def _dot(a, b):
    return jnp.dot(a, b, preferred_element_type=f32)


_LHS = ((2, -1, 0), (2, 1, 3), (3, 0, None), (0, 1, 3), (0, 0, None), (0, 1, 1), (1, -1, 3))
_RHS = ((0, 1, 1), (0, 0, None), (2, -1, 0), (0, 1, 3), (1, -1, 3), (3, 0, None), (2, 1, 3))
_USES = (((3, 1),), ((2, 1), (3, -1)), ((2, 1), (0, 1)), ((0, 1), (3, 1)),
         ((3, 1), (1, 1)), ((1, 1), (0, -1)), ((0, 1),))
_LAST = (6, 5, 2, 4)
_PLAIN = (8, 12, 36, 40)


def _operands(table, g, block):
    def halves(x):
        return x if isinstance(x, (list, tuple)) else [_half(x, 0), _half(x, 1)]

    def comb(x, sign, y):
        return [a + b if sign > 0 else a - b for a, b in zip(halves(x), halves(y))]

    i, sign, j = table[g]
    inner = []
    for r in range(2):
        for c in range(2):
            x = block(2 * (i // 2) + r, 2 * (i % 2) + c)
            inner.append(comb(x, sign, block(2 * (j // 2) + r, 2 * (j % 2) + c)) if sign else x)
    out = []
    for i, sign, j in table:
        x = comb(inner[i], sign, inner[j]) if sign else inner[i]
        out.append(_pack2(*x) if isinstance(x, (list, tuple)) else x)
    return out


def _left7(u):
    r, c = u.shape[0] // 2, u.shape[1] // 2
    x = [u[:r, :c], u[:r, c:], u[r:, :c], u[r:, c:]]
    return [x[i] if not sign else x[i] + x[j] if sign > 0 else x[i] - x[j] for i, sign, j in _LHS]


def _products7(product, emit):
    total = [None] * 4
    for e in range(7):
        m = product(e)
        for q, sign in _USES[e]:
            total[q] = m if total[q] is None else total[q] + m if sign > 0 else total[q] - m
            if e == _LAST[q]:
                emit(q, total[q])
        yield m


def _spread(works, steps, first, last, before=None):
    work = (v for w in works for v in w)
    total, n = steps * len(works), last - first

    def hook(t, result):
        if first <= t < last:
            count = (t + 1 - first) * total // n - (t - first) * total // n
            for k in range(count):
                if before is not None:
                    r = k * result.shape[0] // (8 * count) * 8
                    before(result[r:r + 8, :128])
                next(work)
    return hook


def _tie(zero, ref):
    def write(v):
        rows = pl.ds(pl.multiple_of(ref.shape[-2] - 8 + 8 * zero, 8), 8)
        ref[(zero,) * (len(ref.shape) - 2) + (rows, pl.ds(0, 128))] = pltpu.bitcast(v, ref.dtype)
    return write


def _products49(product, emit, start=None, hooks=(), t0=0):
    total = {}
    for g in range(7):
        def emit_inner(q, v):
            for o, sign in _USES[g]:
                rc = (2 * (o // 2) + q // 2, 2 * (o % 2) + q % 2)
                if rc not in total:
                    total[rc] = v if start is None else start(*rc) + v
                else:
                    total[rc] = total[rc] + v if sign > 0 else total[rc] - v
                if g == _LAST[o]:
                    emit(*rc, total.pop(rc))

        for e, m in enumerate(_products7(lambda e: product(7 * g + e), emit_inner)):
            for hook in hooks:
                hook(t0 + 7 * g + e, m)


def _kernel(x_hbm, mem0_ref, wq_hbm, wk_hbm, wv_hbm, wo_hbm, w1_hbm, w2_hbm,
            w3_hbm, w4_hbm, out_hbm,
            wo_b, hbuf, xg, w1s, w2b, w3b, w4b, sems, zero_ref, stats, *q_rings):
    pl.run_scoped(
        functools.partial(_block_a, x_hbm, mem0_ref, (wq_hbm, wk_hbm, wv_hbm), wo_hbm,
                          w1_hbm, (w2_hbm, w3_hbm, w4_hbm), wo_b, hbuf, xg, w1s,
                          (w2b, w3b, w4b), sems, zero_ref, stats, q_rings),
        [pltpu.VMEM((H, D // 2, DH), u32)] * 3,
        [pltpu.VMEM((H // 8, RING, DH), f32)] * 16,
        pltpu.VMEM((7, TOK, D // 2), u32),
        pltpu.VMEM((D // 2, D), u32),
        pltpu.VMEM((S, D), bf16),
        pltpu.VMEM((UNROLL * TOK, D), f32),
    )
    pl.run_scoped(
        functools.partial(_block_b, out_hbm, wo_b, hbuf, xg,
                          w1s, (w2b, w3b, w4b), sems, zero_ref, stats, q_rings),
        pltpu.VMEM((F // FC, 49, D // 8, 128), u32),
        pltpu.VMEM((49, D // 8, C4), u32),
        pltpu.VMEM((49, F // 8, C4), u32),
        pltpu.VMEM((49, RB // 8, C4), u32),
        pltpu.VMEM((49, RB // 8, C4), u32),
        pltpu.VMEM((RB + 8, D), f32),
        [pltpu.VMEM((4, RB + 8, 128), f32)] * 2,
        pltpu.VMEM((2, RB, D), f32),
        pltpu.VMEM((2, RB, D), bf16),
    )


def _late_copies(w_hbm, w_b, sems):
    return [pltpu.make_async_copy(src.bitcast(u32), dst.at[pl.ds(0, dst.shape[0] - 8)],
                                  sems.at[SEM_W2 + i])
            for i, (src, dst) in enumerate(zip(w_hbm, w_b))]


def _block_a(x_hbm, mem0_ref, w_hbm, wo_hbm, w1_hbm, late_hbm, wo_b, hbuf, xg, w1s,
             late_b, sems, zero_ref, stats, q_rings, w_s, kv_rings, ubuf, w1b, xs, tokbuf):
    rings = list(q_rings) + list(kv_rings)
    ring = [[rings[m * 8 + h % 8].at[h // 8] for h in range(H)] for m in range(3)]
    q_r, k_r, v_r = ring

    def wo_copy(i):
        rows = pl.ds(i * 512, 512)
        return pltpu.make_async_copy(wo_hbm.bitcast(u32).at[rows], wo_b.at[rows],
                                     sems.at[SEM_WO + i])

    w1_copy = pltpu.make_async_copy(w1_hbm.bitcast(u32), w1b, sems.at[SEM_W1])

    x_rest = [pltpu.make_async_copy(x_hbm.at[pl.ds(r0, r1 - r0)], xs.at[pl.ds(r0, r1 - r0)],
                                    sems.at[SEM_XR + i])
              for i, (r0, r1) in enumerate(((P0, X_LATE), (S - P0, S), (X_LATE, S - P0)))]
    other_copies = [wo_copy(i) for i in range(4)] + [w1_copy] + x_rest[:2]

    def prologue(stg, forms, x49):
        def start_chunk(g, m, pairs=range(4), sem=None):
            for pair in pairs:
                pltpu.make_async_copy(
                    w_hbm[m].bitcast(u32).at[:, 4 * g + pair, :], stg[m].at[pl.ds(pair * D, D)],
                    sems.at[SEM_W + 3 * g + m if sem is None else sem]).start()

        def wait_chunk(g, m, rows=pl.ds(0, 4 * D), sem=None):
            pltpu.make_async_copy(stg[m].at[rows], stg[m].at[rows],
                                  sems.at[SEM_W + 3 * g + m if sem is None else sem]).wait()

        def relayout(g, m, half, i):
            for a in range(2):
                ev, od = [stg[m][pl.ds((2 * half + a) * D + 2 * i + par, 8, stride=2), :]
                          for par in range(2)]
                for z in range(2):
                    w_s[m][8 * g + 4 * half + 2 * a + z, pl.ds(i, 8), :] = _pack2(
                        _half(ev, z), _half(od, z))

        def operands(g, m, half, i0, ahead):
            for grp in range(7):
                def word(k, n):
                    return w_s[m][8 * g + 4 * half + n + (g >> (4 + grp // RG)),
                                  pl.ds(k * (D // 8) + i0, 8), :]
                for e, v in enumerate(_operands(_RHS, grp, word)):
                    if 7 * grp + e not in _PLAIN:
                        forms[half + (g >> 2), 7 * grp + e, pl.ds(i0, 8), :] = v
                        yield
                if ahead is not None and grp in RAT:
                    relayout(g, m, half, RAT.index(grp) * (D // 8) + ahead)

        def x_copy(i):
            rows = pl.ds(_mult(i * 128, 128), 128)
            return pltpu.make_async_copy(x_hbm.at[rows], xs.at[rows], sems.at[SEM_X + i])

        start_chunk(0, 0, range(2), SEM_W0)
        for i in range(P0 // 128):
            x_copy(i).start()
        start_chunk(0, 0, range(2, 4))
        for m in range(1, 3):
            start_chunk(0, m)
        zero = jnp.zeros((HALO, 128), f32)
        for c in range(D // 128):
            xg[c, pl.ds(0, HALO), :] = zero
            xg[c, pl.ds(HALO + S, HALO), :] = zero
        hbuf[pl.ds(0, 4 * TOK), :] = jnp.zeros((4 * TOK, D), f32)
        wait_chunk(0, 0, pl.ds(0, 2 * D), SEM_W0)

        @pl.loop(0, D // 64)
        def _(i):
            for k in range(4):
                relayout(0, 0, 0, pl.multiple_of(k * (D // 8) + 8 * i, 8))
            for _ in operands(0, 0, 0, pl.multiple_of(8 * i, 8), None):
                pass

        @pl.loop(0, P0 // 128)
        def _(i):
            x_copy(i).wait()
            r0 = pl.multiple_of(i * 128, 128)
            xn = _ln(xs[pl.ds(r0, 128), :].astype(f32))
            for c in range(D // 128):
                xg[c, pl.ds(HALO + r0, 128), :] = xn[:, c * 128:(c + 1) * 128]

        @pl.loop(0, P0 // 64)
        def _(i):
            for c in range(2):
                def block(a, k):
                    return [xg[2 * k + c, pl.ds(HALO + a * (P0 // 4) + 16 * i + z, 8, stride=2), :]
                            for z in range(2)]
                for grp in range(7):
                    for e, v in enumerate(_operands(_LHS, grp, block)):
                        x49[7 * grp + e, pl.ds(pl.multiple_of(8 * i, 8), 8), pl.ds(128 * c, 128)] = v

        wait_chunk(0, 0, pl.ds(2 * D, 2 * D))

        def stage(g, m, half):
            c = 3 * g + m
            if half == 0:
                g1, m1 = g, m
            else:
                g1, m1 = jnp.minimum(g + (1 if m == 2 else 0), 3), (m + 1) % 3

            def begin(t, _):
                if t != WAT * half:
                    return
                if half == 1:
                    pl.when(g < 3)(functools.partial(start_chunk, g + 1, m))
                    for at, copy in zip(DMA_AT, other_copies):
                        if at % 3 == m:
                            pl.when(g == at // 3)(copy.start)
                    pl.when(c < 11)(functools.partial(wait_chunk, g1, m1))
                for k in range(4):
                    relayout(g1, m1, 1 - half, k * (D // 8))

            hook = _spread([operands(g1, m1, 1 - half, i0, i0 + 8 if i0 + 8 < D // 8 else None)
                            for i0 in range(0, D // 8, 8)], 45, (WAT + 1) * half, 49 * PSUB - PEND)
            rows = P0 // 4 // PSUB
            for sub in range(PSUB):
                zero = g >> (3 + sub + PSUB * (2 * m + half))

                def product(p):
                    if p in _PLAIN:
                        k = _PLAIN.index(p)
                        w = w_s[m][8 * g + 4 * half + k + zero, pl.ds(k * (D // 8), D // 8), :]
                    else:
                        w = forms[half + zero, p]
                    return _dot(_unpack(x49[p + zero, pl.ds(sub * rows // 2, rows // 2), :]),
                                _unpack(w))

                def emit(a, n, v):
                    rings[m * 8 + 4 * half + n][g, pl.ds(a * (P0 // 4) + sub * rows, rows), :] = v

                _products49(product, emit, hooks=[begin, hook], t0=49 * sub)

        @pl.loop(0, 4)
        def _(g):
            for m in range(3):
                for half in range(2):
                    stage(g, m, half)

    pl.run_scoped(
        prologue,
        [pltpu.VMEM((4 * D + 8, DH), u32)] * 3,
        pltpu.VMEM((2, 49, D // 8, DH), u32),
        pltpu.VMEM((49, P0 // 8, C4), u32),
    )
    x_rest[2].start()
    for copy in _late_copies(late_hbm, late_b, sems):
        copy.start()
    for pending in other_copies:
        pending.wait()

    @pl.loop(0, D // 32)
    def _(i):
        for c in range(4):
            x = [w1b[pl.ds(pl.multiple_of(k * (D // 4) + 8 * i, 8), 8),
                     pl.ds(n * (D // 2) + 128 * c, 128)] for k in range(2) for n in range(2)]
            for e, (a, sign, b) in enumerate(_RHS):
                halves = [(_half(x[a], z), _half(x[b], z)) for z in range(2)] if sign else None
                w1s[c, e, pl.ds(pl.multiple_of(8 * i, 8), 8), :] = x[a] if not sign else _pack2(
                    *[u + v if sign > 0 else u - v for u, v in halves])

    def wrap(r):
        return jnp.where(r >= RING, r - RING, r)

    def stage_tokens(i):
        n = UNROLL * TOK
        tokbuf[...] = _ln(xs[pl.ds(_mult(P0 + n * i, 16), n), :].astype(f32))

    def step(s, carry, tok, resid, first_of_group):
        mem, rp, ra, rw = carry
        ri = lax.broadcasted_iota(jnp.int32, (2 * L, 2 * L), 0)
        ci = lax.broadcasted_iota(jnp.int32, (2 * L, 2 * L), 1)
        same = (ri >= L) == (ci >= L)
        mask = same & ((jnp.where(ri >= L, ri - L, ri) < MEM) | (ri >= ci))
        fill = jnp.where(same, NEG, -jnp.inf)

        lhs = jnp.concatenate([mem, tok], axis=0).astype(bf16)
        rps = [pl.multiple_of(wrap(rp + 8 * i), 8) for i in range(3)]
        ra_ = pl.multiple_of(ra, SEG)
        rw_ = pl.multiple_of(rw, 8)

        col = s & 3
        rb = pl.multiple_of(jnp.maximum((s >> 2) - 1, 0) * (4 * TOK), 8)
        if first_of_group:
            u = _ln_twice(hbuf[pl.ds(rb, 4 * TOK), :], stats, pl.ds(rb, 4 * TOK))
            for e, v in enumerate(_left7(u)):
                ubuf[e] = _pack(v)

        def emit(q, v):
            xg[4 * (q % 2) + col, pl.ds(HALO + rb + 2 * TOK * (q // 2), 2 * TOK), :] = _gelu(v)

        fill_work = _products7(lambda e: _dot(_unpack(ubuf[e]), _unpack(w1s[col, e])), emit)

        def filler(j):
            for _ in range((FILL_N, 7 - FILL_N)[j]):
                next(fill_work)

        mem_qkv = {}
        scores = {}
        o_mem = {}
        total = [None]

        def qkv(h):
            res = []
            for m in range(3):
                r = _dot(lhs, _unpack(w_s[m][h]))
                for i in range(3):
                    ring[m][h][pl.ds(rps[i], 8), :] = r[8 + 8 * i:16 + 8 * i]
                res.append(r[:MEM])
            mem_qkv[h] = res

        def both(h, mem_rows, ring_m):
            return jnp.concatenate(
                [x for k in range(2) for x in (mem_rows[k], ring_m[h + k][pl.ds(ra_, SEG), :])],
                axis=0).astype(bf16)

        def qk(h):
            qm, km, vm = zip(mem_qkv.pop(h), mem_qkv.pop(h + 1))
            sc = lax.dot_general(both(h, qm, q_r), both(h, km, k_r), (((1,), (1,)), ((), ())),
                                 preferred_element_type=f32)
            scores[h] = (sc, vm)

        def pv(h):
            sc, vm = scores.pop(h)
            sc = jnp.where(mask, sc * (DH ** -0.5), fill)
            mx = jnp.max(sc, axis=1, keepdims=True)
            e = jnp.exp(sc - mx)
            den = jnp.sum(e, axis=1, keepdims=True)
            inv = pl.reciprocal(den, approx=True)
            inv = inv * (2.0 - den * inv)
            o = _dot(e.astype(bf16), both(h, vm, v_r)) * inv
            for k in range(2):
                q_r[h + k][pl.ds(ra_, SEG), :] = o[k * L + MEM:(k + 1) * L]
                o_mem[h + k] = o[k * L:k * L + MEM]

        def wo(h):
            lo = jnp.concatenate([o_mem.pop(h), q_r[h][pl.ds(rw_, TOK), :]],
                                 axis=0).astype(bf16)
            r = _dot(lo, _unpack(wo_b[pl.ds(h * DH // 2, DH // 2), :]))
            total[0] = r if total[0] is None else total[0] + r

        slot = {"s": (LAG_QK, qk, 0), "p": (LAG_PV, pv, 0), "a": (0, qkv, 0), "b": (0, qkv, 1),
                "x": (LAG_WO, wo, 0), "y": (LAG_WO, wo, 1)}
        for t in range(H // 2 + LAG_WO + 1):
            for kind in ORDER:
                if kind == "f":
                    for j in range(2):
                        if t == H // 2 + LAG_WO - (FILL_AT if first_of_group else FILL_B)[j]:
                            filler(j)
                    continue
                lag, fn, k = slot[kind]
                if 0 <= t - lag < H // 2:
                    fn(2 * (t - lag) + k)

        a = total[0]
        hbuf[pl.ds(pl.multiple_of(TOK * s, 8), TOK), :] = resid + a[MEM:]
        return a[:MEM], wrap(rp + TOK), wrap(ra + SEG), wrap(rw + TOK)

    def steps(i, carry):
        @pl.when(i == NSEG // UNROLL // 2)
        def _():
            for copy in _late_copies(late_hbm, late_b, sems):
                copy.wait()

        n = UNROLL * TOK
        pl.when(i == (X_LATE - P0) // n - 2)(x_rest[2].wait)
        last = pl.ds(pl.multiple_of(S - P0 + P0 * UNROLL // NSEG * i, 16), P0 * UNROLL // NSEG)
        hbuf[last, :] = xs[last, :].astype(f32)
        toks = tokbuf[...]
        resid = xs[pl.ds(pl.multiple_of(n * i, 16), n), :].astype(f32)
        for k in range(UNROLL):
            rows = slice(k * TOK, (k + 1) * TOK)
            carry = step(i * UNROLL + k, carry, toks[rows], resid[rows], k == 0)
            if k == 0:
                stage_tokens(jnp.minimum(i + 1, NSEG // UNROLL - 1))
        return carry

    stage_tokens(0)
    carry = lax.fori_loop(
        0, NSEG // UNROLL, steps,
        (mem0_ref[...].astype(f32), jnp.int32(P0), jnp.int32(0), jnp.int32(0)))
    zero_ref[0] = carry[1] >> 12


def _block_b(out_hbm, wo_b, hbuf, xg, w1s, late_b, sems, zero_ref, stats, q_rings,
             w3s, w2s, w4s, y49, g49, xbuf, tbuf, res, obuf):
    w2b, w3b, w4b = late_b
    nj = F // FC
    Q = RB // 4

    def out_copy(i, cols=pl.ds(0, D), sem=0):
        rows = pl.ds(_mult(i * RB, RB), RB)
        return pltpu.make_async_copy(obuf.at[i & 1, :, cols], out_hbm.at[rows, cols],
                                     sems.at[SEM_OUT + (i & 1) + sem])

    last_copies = [out_copy(S // RB - 1, pl.ds(k * (D // 2), D // 2), k) for k in range(2)]

    def weight_work(src, dst, row, col, at):
        for grp in range(7):
            def word(k, n):
                return src[pl.ds(_mult(row(k), 8), 8), pl.ds(col(n), 128)]
            for e, v in enumerate(_operands(_RHS, grp, word)):
                dst[at(7 * grp + e)] = v
            yield

    def w2_work(i, c):
        return weight_work(w2b, w2s, lambda k: k * (D // 8) + i, lambda n: n * C4 + c,
                           lambda p: (p, pl.ds(_mult(i, 8), 8), pl.ds(c, 128)))

    def w3_work(j, i):
        return weight_work(w3b, w3s, lambda k: k * (D // 8) + i, lambda n: j * FC + n * 128,
                           lambda p: (j, p, pl.ds(_mult(i, 8), 8)))

    def w4_work(j, i, c):
        return weight_work(w4b, w4s, lambda k: j * (FC // 2) + k * 64 + i, lambda n: 4 * c + n * 128,
                           lambda p: (p, pl.ds(_mult(j * 64 + i, 8), 8), pl.ds(c, 128)))

    def gather(pieces, p, cols):
        return _unpack(jnp.concatenate(
            [jnp.concatenate([pieces[c, r][p] for r in range(0, Q, 16)], axis=0)
             for c in cols], axis=1))

    def left_work(dst, block, r, c):
        for grp in range(7):
            for e, v in enumerate(_operands(_LHS, grp, block)):
                dst[7 * grp + e, pl.ds(_mult(r // 2, 8), 8), pl.ds(128 * c, 128)] = v
            yield

    def shift_work(i, r, c):
        def block(a, k):
            r0 = HALO + i * RB + a * Q + r + (-1, 1, -2, 2)[k]
            return [xg[2 * k + c, pl.ds(r0 + z, 8, stride=2), :] for z in range(2)]
        return left_work(g49, block, r, c)

    def y_work(r, c):
        def block(a, k):
            r0 = a * Q + 32 * (r // 32) + (r // 16) % 2
            return [tbuf[c][k, pl.ds(r0 + 2 * z, 8, stride=4), :] for z in range(2)]
        return left_work(y49, block, r, c)

    pieces = [(r, c) for r in range(0, Q, 16) for c in range(2)]

    def mixer_out(i, hooks=()):
        for c in range(0, C4, 128):
            def emit(a, n, v):
                rows, cols = pl.ds(_mult(i * RB + a * Q, Q), Q), pl.ds(n * C4 + c, 128)
                hv = hbuf[rows, cols]
                x1 = (hv - stats[0, rows, :]) * stats[1, rows, :] + v
                xbuf[pl.ds(a * Q, Q), cols] = x1
                res[i & 1, pl.ds(a * Q, Q), cols] = hv + x1

            _products49(lambda p: _dot(_unpack(g49[p]), _unpack(w2s[p, :, pl.ds(c, 128)])),
                        emit, hooks=hooks, t0=49 * c // 128)

    def norm_x1(r):
        y = _ln(xbuf[pl.ds(r, LN_ROWS), :])
        for k in range(D // 128):
            tbuf[k % 2][k // 2, pl.ds(r, LN_ROWS), :] = y[:, k * 128:(k + 1) * 128]
        yield

    def post_hooks(zero, t0, t1, t2):
        return [_spread([norm_x1(r) for r in range(0, RB, LN_ROWS)], 1, t0, t1 - LN_GAP, _tie(zero, xbuf)),
                *[_spread([y_work(r, c) for r in range(0, Q, 16)], 7, t1 + (t2 - t1) * c // 2,
                          t1 + (t2 - t1) * (c + 1) // 2, _tie(zero, tbuf[c])) for c in range(2)]]

    def mlp_block(i, last):
        hidden = {}

        zero = zero_ref[0]

        def hidden_work(j, r):
            def block(a, n):
                r0 = a * Q + 32 * (r // 32) + 8 * ((r // 16) % 2)
                return [tbuf[j % 2][n, pl.ds(r0 + 16 * z, 8), :] for z in range(2)]
            hidden[j, r] = []
            for grp in range(7):
                hidden[j, r] += _operands(_LHS, grp, block)
                yield

        hooks = []
        for j in range(nj):
            def emit_up(a, n, v):
                tbuf[j % 2][n, pl.ds(a * Q, Q), :] = _gelu(v)

            _products49(lambda p: _dot(_unpack(y49[p]), _unpack(w3s[j, p])), emit_up, hooks=hooks)
            span = (H_FROM, H_TO) if j < nj - 1 or not last else (1, EARLY - 1)
            hooks = [_spread([hidden_work(j, r) for r in range(0, Q, 16)], 7, *span,
                             _tie(zero, tbuf[j % 2]))]

        def down(p, c, j0, j1):
            return _dot(gather(hidden, p, range(j0, j1)),
                        _unpack(w4s[p, pl.ds(64 * j0, 64 * (j1 - j0)), pl.ds(c, 128)]))

        early = {}
        if last:
            for p in range(EARLY):
                early[p, 0] = down(p, 0, 0, nj - 1)
                hooks[0](p, early[p, 0])
            hooks = []
        else:
            mixer_out(i + 1, hooks)
            ahead = jnp.minimum(i + 2, S // RB - 1)
            hooks = [_spread([shift_work(ahead, r, c) for r, c in pieces], 7, G_FROM, G_TO,
                             _tie(i >> 3, xg))]
            hooks += post_hooks(i >> 3, 0, Y_FROM, G_FROM)
        for c in range(0, C4, 128):
            def product(p):
                if (p, c) in early:
                    return early.pop((p, c)) + down(p, c, nj - 1, nj)
                return down(p, c, 0, nj)

            def emit(a, n, v):
                obuf[i & 1, pl.ds(a * Q, Q), pl.ds(4 * c + n * 128, 128)] = v.astype(bf16)

            _products49(product, emit,
                        lambda a, n: res[i & 1, pl.ds(a * Q, Q), pl.ds(4 * c + n * 128, 128)],
                        hooks, 49 * c // 128)
            if last:
                last_copies[c // 128].start()

    done = TOK * NSEG
    first = 4 * TOK * (NSEG // 4 - 1)

    @pl.loop(0, H // 8)
    def _(g):
        works = [[w2_work(32 * g + i, c) for i in range(0, 32, 8) for c in range(0, C4, 128)],
                 [shift_work(0, 16 * g, c) for c in range(2)],
                 [w3_work(j, 32 * g + i) for j in range(nj) for i in range(0, 32, 8)],
                 [w4_work(j, 16 * g + i, c) for j in range(nj)
                  for i in range(0, 16, 8) for c in range(0, C4, 128)]]
        per = TK // DH
        calls = P0 // TM * (8 // per) * 8 * TQ - TEND
        ends = [calls * sum(map(len, works[:k])) // sum(map(len, works)) for k in range(5)]
        hooks = [_spread(works[k], 7, ends[k], ends[k + 1], _tie(g >> 2, src))
                 for k, src in enumerate((w2b, xg, w3b, w4b))]
        t = 0
        for r0 in range(done, S, TM):
            rr = r0 % RING
            n = min(TM, RING - rr)
            spans = [(rr, n)] + ([(0, TM - n)] if n < TM else [])
            for k in range(0, 8, per):
                lo = jnp.concatenate(
                    [jnp.concatenate([q_rings[h][g, pl.ds(*span), :] for span in spans], axis=0)
                     for h in range(k, k + per)], axis=1).astype(bf16)
                rows = pl.ds(pl.multiple_of((8 * g + k) * (DH // 2), TK // 2), TK // 2)
                for c in range(0, D, 128):
                    r = _dot(lo, _unpack(wo_b[rows, pl.ds(c, 128)]))
                    for q in range(0, TM, TM // TQ):
                        hbuf[pl.ds(r0 + q, TM // TQ), pl.ds(c, 128)] += r[q:q + TM // TQ]
                        for hook in hooks:
                            hook(t, r[q:q + TM // TQ])
                        t += 1

    zero = zero_ref[0]
    us = {}

    def norm_h(r):
        us[r] = _ln_twice(hbuf[pl.ds(r, LN_ROWS), :], stats, pl.ds(r, LN_ROWS))
        yield

    blocks = [(first, done - first)] + [(r0, UM) for r0 in range(done, S, UM)]
    lead = 2 * 49
    calls = lead + 28 * len(blocks)
    hooks = [_spread([norm_h(r) for r in range(first, S, LN_ROWS)], 1, 0, calls - 28 - ULEAD,
                     _tie(zero, hbuf)),
             _spread([shift_work(1, r, c) for r, c in pieces], 7, lead, calls - 1, _tie(zero, xg))]
    hooks += post_hooks(zero, lead, (lead + calls) // 2, calls - 1)
    mixer_out(0, hooks)
    for b, (r0, n) in enumerate(blocks):
        left = _left7(jnp.concatenate([us.pop(r) for r in range(r0, r0 + n, LN_ROWS)], axis=0))
        for c in range(4):
            def emit(q, v):
                xg[4 * (q % 2) + c, pl.ds(HALO + r0 + n // 2 * (q // 2), n // 2), :] = _gelu(v)

            for e, m in enumerate(_products7(
                    lambda e: _dot(left[e].astype(bf16), _unpack(w1s[c, e])), emit)):
                for hook in hooks:
                    hook(lead + 28 * b + 7 * c + e, m)

    @pl.loop(0, S // RB - 1)
    def _(i):
        mlp_block(i, False)
        out_copy(i).start()
        pl.when(i > 0)(lambda: out_copy(i - 1).wait())

    mlp_block(S // RB - 1, True)
    for pending in [out_copy(S // RB - 2)] + last_copies:
        pending.wait()


@jax.jit
def pallas_sequential_preLN__memory_aug_recurrent_mem_tr__mixer_s_mlp__prompt_kernel(
    A_x: jax.Array,
    A_mem0: jax.Array,
    A_Wq: jax.Array,
    A_Wk: jax.Array,
    A_Wv: jax.Array,
    A_Wo: jax.Array,
    A_seg_len: jax.Array,
    B_x: jax.Array,
    B_w1: jax.Array,
    B_w2: jax.Array,
    B_w3: jax.Array,
    B_w4: jax.Array,
):
    del A_seg_len, B_x
    hbm = pl.BlockSpec(memory_space=pl.ANY)
    vmem = pl.BlockSpec(memory_space=pltpu.VMEM)
    scratch = [
        pltpu.VMEM((H * DH // 2, D), u32),
        pltpu.VMEM((S + 8, D), f32),
        pltpu.VMEM((D // 128, S + 2 * HALO + 8, 128), f32),
        pltpu.VMEM((4, 7, D // 4, 128), u32),
        pltpu.VMEM((D // 2 + 8, D), u32),
        pltpu.VMEM((D // 2 + 8, F), u32),
        pltpu.VMEM((F // 2 + 8, D), u32),
        pltpu.SemaphoreType.DMA((NSEM,)),
        pltpu.SMEM((1,), jnp.int32),
        pltpu.VMEM((2, S, 128), f32),
    ] + [pltpu.VMEM((H // 8, RING, DH), f32)] * 8
    out = pl.pallas_call(
        _kernel,
        out_shape=jax.ShapeDtypeStruct((S, D), A_x.dtype),
        in_specs=[hbm, vmem] + [hbm] * 8,
        out_specs=hbm,
        scratch_shapes=scratch,
        compiler_params=pltpu.CompilerParams(vmem_limit_bytes=255 * 512 * 1024),
    )(A_x.reshape(S, D), A_mem0.reshape(MEM, D),
      A_Wq, A_Wk, A_Wv,
      A_Wo.reshape(H * DH, D), B_w1, B_w2, B_w3, B_w4)
    return out.reshape(A_x.shape)
```

```python
import functools

import jax
import jax.numpy as jnp
from jax import lax
import jax.experimental.pallas as pl
import jax.experimental.pallas.tpu as pltpu

S = 2048
D = 1024
H = 32
DH = 128
MEM = 8
SEG = 32
F = 3584
NSEG = S // SEG
L = MEM + SEG
TOK = 24
P0 = S - TOK * NSEG
RING = 576
C4 = D // 4
HALO = 8
RB = 256
FC = 512
EPS = 1e-5
NEG = -1000000000.0

X_LATE = 704

PSUB = 2
WAT = 1
PEND = 2
RG = 4
RAT = (0, 1, 4, 5)
DMA_AT = (2, 4, 6, 9, 8, 9, 9)

LAG_QK = 2
LAG_PV = 4
LAG_WO = 5
ORDER = "pbsafxy"
FILL_AT = (4, 0)
FILL_B = (4, 4)
FILL_N = 1
UNROLL = 2

TM = 128
TK = 512
TQ = 8
TEND = 8
UM = 64
ULEAD = 120
LN_ROWS = 8
LN_GAP = 1
Y_FROM = 42
G_FROM = 72
G_TO = 97
H_FROM = 4
H_TO = 48
EARLY = 16

bf16 = jnp.bfloat16
f32 = jnp.float32
u32 = jnp.uint32

SEM_X, SEM_XR, SEM_WO, SEM_W1, SEM_W2, SEM_OUT, SEM_W0, SEM_W = 0, 4, 7, 11, 15, 18, 21, 22
NSEM = SEM_W + 12


def _mult(i, n):
    return i if isinstance(i, int) else pl.multiple_of(i, n)


def _ln(x):
    m = jnp.mean(x, axis=-1, keepdims=True)
    d = x - m
    v = jnp.mean(d * d, axis=-1, keepdims=True)
    return d * lax.rsqrt(v + EPS)


def _ln_twice(x, stats, rows):
    m = jnp.mean(x, axis=-1, keepdims=True)
    d = x - m
    scale = lax.rsqrt(jnp.mean(d * d, axis=-1, keepdims=True) + EPS)
    for k, v in enumerate((m, scale)):
        stats[k, rows, :] = jnp.broadcast_to(v, (x.shape[0], 128))
    return _ln(d * scale)


def _gelu(x):
    return jax.nn.gelu(x, approximate=True)


def _pack(x):
    return pltpu.bitcast(x.astype(bf16), u32)


def _unpack(x):
    return pltpu.bitcast(x, bf16)


def _pack2(even, odd):
    lo, hi = [pltpu.bitcast(x, u32) + jnp.uint32(0x8000) for x in (even, odd)]
    return (lo >> 16) | (hi & jnp.uint32(0xFFFF0000))


def _half(w, i):
    return pltpu.bitcast(w & jnp.uint32(0xFFFF0000) if i else w << 16, f32)


def _dot(a, b):
    return jnp.dot(a, b, preferred_element_type=f32)


_LHS = ((2, -1, 0), (2, 1, 3), (3, 0, None), (0, 1, 3), (0, 0, None), (0, 1, 1), (1, -1, 3))
_RHS = ((0, 1, 1), (0, 0, None), (2, -1, 0), (0, 1, 3), (1, -1, 3), (3, 0, None), (2, 1, 3))
_USES = (((3, 1),), ((2, 1), (3, -1)), ((2, 1), (0, 1)), ((0, 1), (3, 1)),
         ((3, 1), (1, 1)), ((1, 1), (0, -1)), ((0, 1),))
_LAST = (6, 5, 2, 4)
_PLAIN = (8, 12, 36, 40)


def _operands(table, g, block):
    def halves(x):
        return x if isinstance(x, (list, tuple)) else [_half(x, 0), _half(x, 1)]

    def comb(x, sign, y):
        return [a + b if sign > 0 else a - b for a, b in zip(halves(x), halves(y))]

    i, sign, j = table[g]
    inner = []
    for r in range(2):
        for c in range(2):
            x = block(2 * (i // 2) + r, 2 * (i % 2) + c)
            inner.append(comb(x, sign, block(2 * (j // 2) + r, 2 * (j % 2) + c)) if sign else x)
    out = []
    for i, sign, j in table:
        x = comb(inner[i], sign, inner[j]) if sign else inner[i]
        out.append(_pack2(*x) if isinstance(x, (list, tuple)) else x)
    return out


def _left7(u):
    r, c = u.shape[0] // 2, u.shape[1] // 2
    x = [u[:r, :c], u[:r, c:], u[r:, :c], u[r:, c:]]
    return [x[i] if not sign else x[i] + x[j] if sign > 0 else x[i] - x[j] for i, sign, j in _LHS]


def _products7(product, emit):
    total = [None] * 4
    for e in range(7):
        m = product(e)
        for q, sign in _USES[e]:
            total[q] = m if total[q] is None else total[q] + m if sign > 0 else total[q] - m
            if e == _LAST[q]:
                emit(q, total[q])
        yield m


def _spread(works, steps, first, last, before=None):
    work = (v for w in works for v in w)
    total, n = steps * len(works), last - first

    def hook(t, result):
        if first <= t < last:
            count = (t + 1 - first) * total // n - (t - first) * total // n
            for k in range(count):
                if before is not None:
                    r = k * result.shape[0] // (8 * count) * 8
                    before(result[r:r + 8, :128])
                next(work)
    return hook


def _tie(zero, ref):
    def write(v):
        rows = pl.ds(pl.multiple_of(ref.shape[-2] - 8 + 8 * zero, 8), 8)
        ref[(zero,) * (len(ref.shape) - 2) + (rows, pl.ds(0, 128))] = pltpu.bitcast(v, ref.dtype)
    return write


def _products49(product, emit, start=None, hooks=(), t0=0):
    total = {}
    for g in range(7):
        def emit_inner(q, v):
            for o, sign in _USES[g]:
                rc = (2 * (o // 2) + q // 2, 2 * (o % 2) + q % 2)
                if rc not in total:
                    total[rc] = v if start is None else start(*rc) + v
                else:
                    total[rc] = total[rc] + v if sign > 0 else total[rc] - v
                if g == _LAST[o]:
                    emit(*rc, total.pop(rc))

        for e, m in enumerate(_products7(lambda e: product(7 * g + e), emit_inner)):
            for hook in hooks:
                hook(t0 + 7 * g + e, m)


def _kernel(x_hbm, mem0_ref, wq_hbm, wk_hbm, wv_hbm, wo_hbm, w1_hbm, w2_hbm,
            w3_hbm, w4_hbm, out_hbm,
            wo_b, hbuf, xg, w1s, w2b, w3b, w4b, sems, zero_ref, stats, *q_rings):
    pl.run_scoped(
        functools.partial(_block_a, x_hbm, mem0_ref, (wq_hbm, wk_hbm, wv_hbm), wo_hbm,
                          w1_hbm, (w2_hbm, w3_hbm, w4_hbm), wo_b, hbuf, xg, w1s,
                          (w2b, w3b, w4b), sems, zero_ref, stats, q_rings),
        [pltpu.VMEM((H, D // 2, DH), u32)] * 3,
        [pltpu.VMEM((H // 8, RING, DH), f32)] * 16,
        pltpu.VMEM((7, TOK, D // 2), u32),
        pltpu.VMEM((D // 2, D), u32),
        pltpu.VMEM((S, D), bf16),
        pltpu.VMEM((UNROLL * TOK, D), f32),
    )
    pl.run_scoped(
        functools.partial(_block_b, out_hbm, wo_b, hbuf, xg,
                          w1s, (w2b, w3b, w4b), sems, zero_ref, stats, q_rings),
        pltpu.VMEM((F // FC, 49, D // 8, 128), u32),
        pltpu.VMEM((49, D // 8, C4), u32),
        pltpu.VMEM((49, F // 8, C4), u32),
        pltpu.VMEM((49, RB // 8, C4), u32),
        pltpu.VMEM((49, RB // 8, C4), u32),
        pltpu.VMEM((RB + 8, D), f32),
        [pltpu.VMEM((4, RB + 8, 128), f32)] * 2,
        pltpu.VMEM((2, RB, D), f32),
        pltpu.VMEM((2, RB, D), bf16),
    )


def _late_copies(w_hbm, w_b, sems):
    return [pltpu.make_async_copy(src.bitcast(u32), dst.at[pl.ds(0, dst.shape[0] - 8)],
                                  sems.at[SEM_W2 + i])
            for i, (src, dst) in enumerate(zip(w_hbm, w_b))]


def _block_a(x_hbm, mem0_ref, w_hbm, wo_hbm, w1_hbm, late_hbm, wo_b, hbuf, xg, w1s,
             late_b, sems, zero_ref, stats, q_rings, w_s, kv_rings, ubuf, w1b, xs, tokbuf):
    rings = list(q_rings) + list(kv_rings)
    ring = [[rings[m * 8 + h % 8].at[h // 8] for h in range(H)] for m in range(3)]
    q_r, k_r, v_r = ring

    def wo_copy(i):
        rows = pl.ds(i * 512, 512)
        return pltpu.make_async_copy(wo_hbm.bitcast(u32).at[rows], wo_b.at[rows],
                                     sems.at[SEM_WO + i])

    w1_copy = pltpu.make_async_copy(w1_hbm.bitcast(u32), w1b, sems.at[SEM_W1])

    x_rest = [pltpu.make_async_copy(x_hbm.at[pl.ds(r0, r1 - r0)], xs.at[pl.ds(r0, r1 - r0)],
                                    sems.at[SEM_XR + i])
              for i, (r0, r1) in enumerate(((P0, X_LATE), (S - P0, S), (X_LATE, S - P0)))]
    other_copies = [wo_copy(i) for i in range(4)] + [w1_copy] + x_rest[:2]

    def prologue(stg, forms, x49):
        def start_chunk(g, m, pairs=range(4), sem=None):
            for pair in pairs:
                pltpu.make_async_copy(
                    w_hbm[m].bitcast(u32).at[:, 4 * g + pair, :], stg[m].at[pl.ds(pair * D, D)],
                    sems.at[SEM_W + 3 * g + m if sem is None else sem]).start()

        def wait_chunk(g, m, rows=pl.ds(0, 4 * D), sem=None):
            pltpu.make_async_copy(stg[m].at[rows], stg[m].at[rows],
                                  sems.at[SEM_W + 3 * g + m if sem is None else sem]).wait()

        def relayout(g, m, half, i):
            for a in range(2):
                ev, od = [stg[m][pl.ds((2 * half + a) * D + 2 * i + par, 8, stride=2), :]
                          for par in range(2)]
                h = 8 * g + 4 * half + 2 * a
                w_s[m][h, pl.ds(i, 8), :] = (ev & jnp.uint32(0xFFFF)) | (od << 16)
                w_s[m][h + 1, pl.ds(i, 8), :] = (ev >> 16) | (od & jnp.uint32(0xFFFF0000))

        def operands(g, m, half, i0, ahead):
            for grp in range(7):
                def word(k, n):
                    return w_s[m][8 * g + 4 * half + n + (g >> (4 + grp // RG)),
                                  pl.ds(k * (D // 8) + i0, 8), :]
                for e, v in enumerate(_operands(_RHS, grp, word)):
                    if 7 * grp + e not in _PLAIN:
                        forms[half + (g >> 2), 7 * grp + e, pl.ds(i0, 8), :] = v
                        yield
                if ahead is not None and grp in RAT:
                    relayout(g, m, half, RAT.index(grp) * (D // 8) + ahead)

        def x_copy(i):
            rows = pl.ds(_mult(i * 128, 128), 128)
            return pltpu.make_async_copy(x_hbm.at[rows], xs.at[rows], sems.at[SEM_X + i])

        start_chunk(0, 0, range(2), SEM_W0)
        for i in range(P0 // 128):
            x_copy(i).start()
        start_chunk(0, 0, range(2, 4))
        for m in range(1, 3):
            start_chunk(0, m)
        zero = jnp.zeros((HALO, 128), f32)
        for c in range(D // 128):
            xg[c, pl.ds(0, HALO), :] = zero
            xg[c, pl.ds(HALO + S, HALO), :] = zero
        hbuf[pl.ds(0, 4 * TOK), :] = jnp.zeros((4 * TOK, D), f32)
        wait_chunk(0, 0, pl.ds(0, 2 * D), SEM_W0)

        @pl.loop(0, D // 64)
        def _(i):
            for k in range(4):
                relayout(0, 0, 0, pl.multiple_of(k * (D // 8) + 8 * i, 8))
            for _ in operands(0, 0, 0, pl.multiple_of(8 * i, 8), None):
                pass

        @pl.loop(0, P0 // 128)
        def _(i):
            x_copy(i).wait()
            r0 = pl.multiple_of(i * 128, 128)
            xn = _ln(xs[pl.ds(r0, 128), :].astype(f32))
            for c in range(D // 128):
                xg[c, pl.ds(HALO + r0, 128), :] = xn[:, c * 128:(c + 1) * 128]

        @pl.loop(0, P0 // 64)
        def _(i):
            for c in range(2):
                def block(a, k):
                    return [xg[2 * k + c, pl.ds(HALO + a * (P0 // 4) + 16 * i + z, 8, stride=2), :]
                            for z in range(2)]
                for grp in range(7):
                    for e, v in enumerate(_operands(_LHS, grp, block)):
                        x49[7 * grp + e, pl.ds(pl.multiple_of(8 * i, 8), 8), pl.ds(128 * c, 128)] = v

        wait_chunk(0, 0, pl.ds(2 * D, 2 * D))

        def stage(g, m, half):
            c = 3 * g + m
            if half == 0:
                g1, m1 = g, m
            else:
                g1, m1 = jnp.minimum(g + (1 if m == 2 else 0), 3), (m + 1) % 3

            def begin(t, _):
                if t != WAT * half:
                    return
                if half == 1:
                    pl.when(g < 3)(functools.partial(start_chunk, g + 1, m))
                    for at, copy in zip(DMA_AT, other_copies):
                        if at % 3 == m:
                            pl.when(g == at // 3)(copy.start)
                    pl.when(c < 11)(functools.partial(wait_chunk, g1, m1))
                for k in range(4):
                    relayout(g1, m1, 1 - half, k * (D // 8))

            hook = _spread([operands(g1, m1, 1 - half, i0, i0 + 8 if i0 + 8 < D // 8 else None)
                            for i0 in range(0, D // 8, 8)], 45, (WAT + 1) * half, 49 * PSUB - PEND)
            rows = P0 // 4 // PSUB
            for sub in range(PSUB):
                zero = g >> (3 + sub + PSUB * (2 * m + half))

                def product(p):
                    if p in _PLAIN:
                        k = _PLAIN.index(p)
                        w = w_s[m][8 * g + 4 * half + k + zero, pl.ds(k * (D // 8), D // 8), :]
                    else:
                        w = forms[half + zero, p]
                    return _dot(_unpack(x49[p + zero, pl.ds(sub * rows // 2, rows // 2), :]),
                                _unpack(w))

                def emit(a, n, v):
                    rings[m * 8 + 4 * half + n][g, pl.ds(a * (P0 // 4) + sub * rows, rows), :] = v

                _products49(product, emit, hooks=[begin, hook], t0=49 * sub)

        @pl.loop(0, 4)
        def _(g):
            for m in range(3):
                for half in range(2):
                    stage(g, m, half)

    pl.run_scoped(
        prologue,
        [pltpu.VMEM((4 * D + 8, DH), u32)] * 3,
        pltpu.VMEM((2, 49, D // 8, DH), u32),
        pltpu.VMEM((49, P0 // 8, C4), u32),
    )
    x_rest[2].start()
    for copy in _late_copies(late_hbm, late_b, sems):
        copy.start()
    for pending in other_copies:
        pending.wait()

    @pl.loop(0, D // 32)
    def _(i):
        for c in range(4):
            x = [w1b[pl.ds(pl.multiple_of(k * (D // 4) + 8 * i, 8), 8),
                     pl.ds(n * (D // 2) + 128 * c, 128)] for k in range(2) for n in range(2)]
            for e, (a, sign, b) in enumerate(_RHS):
                halves = [(_half(x[a], z), _half(x[b], z)) for z in range(2)] if sign else None
                w1s[c, e, pl.ds(pl.multiple_of(8 * i, 8), 8), :] = x[a] if not sign else _pack2(
                    *[u + v if sign > 0 else u - v for u, v in halves])

    def wrap(r):
        return jnp.where(r >= RING, r - RING, r)

    def stage_tokens(i):
        n = UNROLL * TOK
        tokbuf[...] = _ln(xs[pl.ds(_mult(P0 + n * i, 16), n), :].astype(f32))

    def step(s, carry, tok, resid, first_of_group):
        mem, rp, ra, rw = carry
        ri = lax.broadcasted_iota(jnp.int32, (2 * L, 2 * L), 0)
        ci = lax.broadcasted_iota(jnp.int32, (2 * L, 2 * L), 1)
        same = (ri >= L) == (ci >= L)
        mask = same & ((jnp.where(ri >= L, ri - L, ri) < MEM) | (ri >= ci))
        fill = jnp.where(same, NEG, -jnp.inf)

        lhs = jnp.concatenate([mem, tok], axis=0).astype(bf16)
        rps = [pl.multiple_of(wrap(rp + 8 * i), 8) for i in range(3)]
        ra_ = pl.multiple_of(ra, SEG)
        rw_ = pl.multiple_of(rw, 8)

        col = s & 3
        rb = pl.multiple_of(jnp.maximum((s >> 2) - 1, 0) * (4 * TOK), 8)
        if first_of_group:
            u = _ln_twice(hbuf[pl.ds(rb, 4 * TOK), :], stats, pl.ds(rb, 4 * TOK))
            for e, v in enumerate(_left7(u)):
                ubuf[e] = _pack(v)

        def emit(q, v):
            xg[4 * (q % 2) + col, pl.ds(HALO + rb + 2 * TOK * (q // 2), 2 * TOK), :] = _gelu(v)

        fill_work = _products7(lambda e: _dot(_unpack(ubuf[e]), _unpack(w1s[col, e])), emit)

        def filler(j):
            for _ in range((FILL_N, 7 - FILL_N)[j]):
                next(fill_work)

        mem_qkv = {}
        scores = {}
        o_mem = {}
        total = [None]

        def qkv(h):
            res = []
            for m in range(3):
                r = _dot(lhs, _unpack(w_s[m][h]))
                for i in range(3):
                    ring[m][h][pl.ds(rps[i], 8), :] = r[8 + 8 * i:16 + 8 * i]
                res.append(r[:MEM])
            mem_qkv[h] = res

        def both(h, mem_rows, ring_m):
            return jnp.concatenate(
                [x for k in range(2) for x in (mem_rows[k], ring_m[h + k][pl.ds(ra_, SEG), :])],
                axis=0).astype(bf16)

        def qk(h):
            qm, km, vm = zip(mem_qkv.pop(h), mem_qkv.pop(h + 1))
            sc = lax.dot_general(both(h, qm, q_r), both(h, km, k_r), (((1,), (1,)), ((), ())),
                                 preferred_element_type=f32)
            scores[h] = (sc, vm)

        def pv(h):
            sc, vm = scores.pop(h)
            sc = jnp.where(mask, sc * (DH ** -0.5), fill)
            mx = jnp.max(sc, axis=1, keepdims=True)
            e = jnp.exp(sc - mx)
            den = jnp.sum(e, axis=1, keepdims=True)
            inv = pl.reciprocal(den, approx=True)
            inv = inv * (2.0 - den * inv)
            o = _dot(e.astype(bf16), both(h, vm, v_r)) * inv
            for k in range(2):
                q_r[h + k][pl.ds(ra_, SEG), :] = o[k * L + MEM:(k + 1) * L]
                o_mem[h + k] = o[k * L:k * L + MEM]

        def wo(h):
            lo = jnp.concatenate([o_mem.pop(h), q_r[h][pl.ds(rw_, TOK), :]],
                                 axis=0).astype(bf16)
            r = _dot(lo, _unpack(wo_b[pl.ds(h * DH // 2, DH // 2), :]))
            total[0] = r if total[0] is None else total[0] + r

        slot = {"s": (LAG_QK, qk, 0), "p": (LAG_PV, pv, 0), "a": (0, qkv, 0), "b": (0, qkv, 1),
                "x": (LAG_WO, wo, 0), "y": (LAG_WO, wo, 1)}
        for t in range(H // 2 + LAG_WO + 1):
            for kind in ORDER:
                if kind == "f":
                    for j in range(2):
                        if t == H // 2 + LAG_WO - (FILL_AT if first_of_group else FILL_B)[j]:
                            filler(j)
                    continue
                lag, fn, k = slot[kind]
                if 0 <= t - lag < H // 2:
                    fn(2 * (t - lag) + k)

        a = total[0]
        hbuf[pl.ds(pl.multiple_of(TOK * s, 8), TOK), :] = resid + a[MEM:]
        return a[:MEM], wrap(rp + TOK), wrap(ra + SEG), wrap(rw + TOK)

    def steps(i, carry):
        @pl.when(i == NSEG // UNROLL // 2)
        def _():
            for copy in _late_copies(late_hbm, late_b, sems):
                copy.wait()

        n = UNROLL * TOK
        pl.when(i == (X_LATE - P0) // n - 2)(x_rest[2].wait)
        last = pl.ds(pl.multiple_of(S - P0 + P0 * UNROLL // NSEG * i, 16), P0 * UNROLL // NSEG)
        hbuf[last, :] = xs[last, :].astype(f32)
        toks = tokbuf[...]
        resid = xs[pl.ds(pl.multiple_of(n * i, 16), n), :].astype(f32)
        for k in range(UNROLL):
            rows = slice(k * TOK, (k + 1) * TOK)
            carry = step(i * UNROLL + k, carry, toks[rows], resid[rows], k == 0)
            if k == 0:
                stage_tokens(jnp.minimum(i + 1, NSEG // UNROLL - 1))
        return carry

    stage_tokens(0)
    carry = lax.fori_loop(
        0, NSEG // UNROLL, steps,
        (mem0_ref[...].astype(f32), jnp.int32(P0), jnp.int32(0), jnp.int32(0)))
    zero_ref[0] = carry[1] >> 12


def _block_b(out_hbm, wo_b, hbuf, xg, w1s, late_b, sems, zero_ref, stats, q_rings,
             w3s, w2s, w4s, y49, g49, xbuf, tbuf, res, obuf):
    w2b, w3b, w4b = late_b
    nj = F // FC
    Q = RB // 4

    def out_copy(i, cols=pl.ds(0, D), sem=0):
        rows = pl.ds(_mult(i * RB, RB), RB)
        return pltpu.make_async_copy(obuf.at[i & 1, :, cols], out_hbm.at[rows, cols],
                                     sems.at[SEM_OUT + (i & 1) + sem])

    last_copies = [out_copy(S // RB - 1, pl.ds(k * (D // 2), D // 2), k) for k in range(2)]

    def weight_work(src, dst, row, col, at):
        for grp in range(7):
            def word(k, n):
                return src[pl.ds(_mult(row(k), 8), 8), pl.ds(col(n), 128)]
            for e, v in enumerate(_operands(_RHS, grp, word)):
                dst[at(7 * grp + e)] = v
            yield

    def w2_work(i, c):
        return weight_work(w2b, w2s, lambda k: k * (D // 8) + i, lambda n: n * C4 + c,
                           lambda p: (p, pl.ds(_mult(i, 8), 8), pl.ds(c, 128)))

    def w3_work(j, i):
        return weight_work(w3b, w3s, lambda k: k * (D // 8) + i, lambda n: j * FC + n * 128,
                           lambda p: (j, p, pl.ds(_mult(i, 8), 8)))

    def w4_work(j, i, c):
        return weight_work(w4b, w4s, lambda k: j * (FC // 2) + k * 64 + i, lambda n: 4 * c + n * 128,
                           lambda p: (p, pl.ds(_mult(j * 64 + i, 8), 8), pl.ds(c, 128)))

    def gather(pieces, p, cols):
        return _unpack(jnp.concatenate(
            [jnp.concatenate([pieces[c, r][p] for r in range(0, Q, 16)], axis=0)
             for c in cols], axis=1))

    def left_work(dst, block, r, c):
        for grp in range(7):
            for e, v in enumerate(_operands(_LHS, grp, block)):
                dst[7 * grp + e, pl.ds(_mult(r // 2, 8), 8), pl.ds(128 * c, 128)] = v
            yield

    def shift_work(i, r, c):
        def block(a, k):
            r0 = HALO + i * RB + a * Q + r + (-1, 1, -2, 2)[k]
            return [xg[2 * k + c, pl.ds(r0 + z, 8, stride=2), :] for z in range(2)]
        return left_work(g49, block, r, c)

    def y_work(r, c):
        def block(a, k):
            r0 = a * Q + 32 * (r // 32) + (r // 16) % 2
            return [tbuf[c][k, pl.ds(r0 + 2 * z, 8, stride=4), :] for z in range(2)]
        return left_work(y49, block, r, c)

    pieces = [(r, c) for r in range(0, Q, 16) for c in range(2)]

    def mixer_out(i, hooks=()):
        for c in range(0, C4, 128):
            def emit(a, n, v):
                rows, cols = pl.ds(_mult(i * RB + a * Q, Q), Q), pl.ds(n * C4 + c, 128)
                hv = hbuf[rows, cols]
                x1 = (hv - stats[0, rows, :]) * stats[1, rows, :] + v
                xbuf[pl.ds(a * Q, Q), cols] = x1
                res[i & 1, pl.ds(a * Q, Q), cols] = hv + x1

            _products49(lambda p: _dot(_unpack(g49[p]), _unpack(w2s[p, :, pl.ds(c, 128)])),
                        emit, hooks=hooks, t0=49 * c // 128)

    def norm_x1(r):
        y = _ln(xbuf[pl.ds(r, LN_ROWS), :])
        for k in range(D // 128):
            tbuf[k % 2][k // 2, pl.ds(r, LN_ROWS), :] = y[:, k * 128:(k + 1) * 128]
        yield

    def post_hooks(zero, t0, t1, t2):
        return [_spread([norm_x1(r) for r in range(0, RB, LN_ROWS)], 1, t0, t1 - LN_GAP, _tie(zero, xbuf)),
                *[_spread([y_work(r, c) for r in range(0, Q, 16)], 7, t1 + (t2 - t1) * c // 2,
                          t1 + (t2 - t1) * (c + 1) // 2, _tie(zero, tbuf[c])) for c in range(2)]]

    def mlp_block(i, last):
        hidden = {}

        zero = zero_ref[0]

        def hidden_work(j, r):
            def block(a, n):
                r0 = a * Q + 32 * (r // 32) + 8 * ((r // 16) % 2)
                return [tbuf[j % 2][n, pl.ds(r0 + 16 * z, 8), :] for z in range(2)]
            hidden[j, r] = []
            for grp in range(7):
                hidden[j, r] += _operands(_LHS, grp, block)
                yield

        hooks = []
        for j in range(nj):
            def emit_up(a, n, v):
                tbuf[j % 2][n, pl.ds(a * Q, Q), :] = _gelu(v)

            _products49(lambda p: _dot(_unpack(y49[p]), _unpack(w3s[j, p])), emit_up, hooks=hooks)
            span = (H_FROM, H_TO) if j < nj - 1 or not last else (1, EARLY - 1)
            hooks = [_spread([hidden_work(j, r) for r in range(0, Q, 16)], 7, *span,
                             _tie(zero, tbuf[j % 2]))]

        def down(p, c, j0, j1):
            return _dot(gather(hidden, p, range(j0, j1)),
                        _unpack(w4s[p, pl.ds(64 * j0, 64 * (j1 - j0)), pl.ds(c, 128)]))

        early = {}
        if last:
            for p in range(EARLY):
                early[p, 0] = down(p, 0, 0, nj - 1)
                hooks[0](p, early[p, 0])
            hooks = []
        else:
            mixer_out(i + 1, hooks)
            ahead = jnp.minimum(i + 2, S // RB - 1)
            hooks = [_spread([shift_work(ahead, r, c) for r, c in pieces], 7, G_FROM, G_TO,
                             _tie(i >> 3, xg))]
            hooks += post_hooks(i >> 3, 0, Y_FROM, G_FROM)
        for c in range(0, C4, 128):
            def product(p):
                if (p, c) in early:
                    return early.pop((p, c)) + down(p, c, nj - 1, nj)
                return down(p, c, 0, nj)

            def emit(a, n, v):
                obuf[i & 1, pl.ds(a * Q, Q), pl.ds(4 * c + n * 128, 128)] = v.astype(bf16)

            _products49(product, emit,
                        lambda a, n: res[i & 1, pl.ds(a * Q, Q), pl.ds(4 * c + n * 128, 128)],
                        hooks, 49 * c // 128)
            if last:
                last_copies[c // 128].start()

    done = TOK * NSEG
    first = 4 * TOK * (NSEG // 4 - 1)

    @pl.loop(0, H // 8)
    def _(g):
        works = [[w2_work(32 * g + i, c) for i in range(0, 32, 8) for c in range(0, C4, 128)],
                 [shift_work(0, 16 * g, c) for c in range(2)],
                 [w3_work(j, 32 * g + i) for j in range(nj) for i in range(0, 32, 8)],
                 [w4_work(j, 16 * g + i, c) for j in range(nj)
                  for i in range(0, 16, 8) for c in range(0, C4, 128)]]
        per = TK // DH
        calls = P0 // TM * (8 // per) * 8 * TQ - TEND
        ends = [calls * sum(map(len, works[:k])) // sum(map(len, works)) for k in range(5)]
        hooks = [_spread(works[k], 7, ends[k], ends[k + 1], _tie(g >> 2, src))
                 for k, src in enumerate((w2b, xg, w3b, w4b))]
        t = 0
        for r0 in range(done, S, TM):
            rr = r0 % RING
            n = min(TM, RING - rr)
            spans = [(rr, n)] + ([(0, TM - n)] if n < TM else [])
            for k in range(0, 8, per):
                lo = jnp.concatenate(
                    [jnp.concatenate([q_rings[h][g, pl.ds(*span), :] for span in spans], axis=0)
                     for h in range(k, k + per)], axis=1).astype(bf16)
                rows = pl.ds(pl.multiple_of((8 * g + k) * (DH // 2), TK // 2), TK // 2)
                for c in range(0, D, 128):
                    r = _dot(lo, _unpack(wo_b[rows, pl.ds(c, 128)]))
                    for q in range(0, TM, TM // TQ):
                        hbuf[pl.ds(r0 + q, TM // TQ), pl.ds(c, 128)] += r[q:q + TM // TQ]
                        for hook in hooks:
                            hook(t, r[q:q + TM // TQ])
                        t += 1

    zero = zero_ref[0]
    us = {}

    def norm_h(r):
        us[r] = _ln_twice(hbuf[pl.ds(r, LN_ROWS), :], stats, pl.ds(r, LN_ROWS))
        yield

    blocks = [(first, done - first)] + [(r0, UM) for r0 in range(done, S, UM)]
    lead = 2 * 49
    calls = lead + 28 * len(blocks)
    hooks = [_spread([norm_h(r) for r in range(first, S, LN_ROWS)], 1, 0, calls - 28 - ULEAD,
                     _tie(zero, hbuf)),
             _spread([shift_work(1, r, c) for r, c in pieces], 7, lead, calls - 1, _tie(zero, xg))]
    hooks += post_hooks(zero, lead, (lead + calls) // 2, calls - 1)
    mixer_out(0, hooks)
    for b, (r0, n) in enumerate(blocks):
        left = _left7(jnp.concatenate([us.pop(r) for r in range(r0, r0 + n, LN_ROWS)], axis=0))
        for c in range(4):
            def emit(q, v):
                xg[4 * (q % 2) + c, pl.ds(HALO + r0 + n // 2 * (q // 2), n // 2), :] = _gelu(v)

            for e, m in enumerate(_products7(
                    lambda e: _dot(left[e].astype(bf16), _unpack(w1s[c, e])), emit)):
                for hook in hooks:
                    hook(lead + 28 * b + 7 * c + e, m)

    @pl.loop(0, S // RB - 1)
    def _(i):
        mlp_block(i, False)
        out_copy(i).start()
        pl.when(i > 0)(lambda: out_copy(i - 1).wait())

    mlp_block(S // RB - 1, True)
    for pending in [out_copy(S // RB - 2)] + last_copies:
        pending.wait()


@jax.jit
def pallas_sequential_preLN__memory_aug_recurrent_mem_tr__mixer_s_mlp__prompt_kernel(
    A_x: jax.Array,
    A_mem0: jax.Array,
    A_Wq: jax.Array,
    A_Wk: jax.Array,
    A_Wv: jax.Array,
    A_Wo: jax.Array,
    A_seg_len: jax.Array,
    B_x: jax.Array,
    B_w1: jax.Array,
    B_w2: jax.Array,
    B_w3: jax.Array,
    B_w4: jax.Array,
):
    del A_seg_len, B_x
    hbm = pl.BlockSpec(memory_space=pl.ANY)
    vmem = pl.BlockSpec(memory_space=pltpu.VMEM)
    scratch = [
        pltpu.VMEM((H * DH // 2, D), u32),
        pltpu.VMEM((S + 8, D), f32),
        pltpu.VMEM((D // 128, S + 2 * HALO + 8, 128), f32),
        pltpu.VMEM((4, 7, D // 4, 128), u32),
        pltpu.VMEM((D // 2 + 8, D), u32),
        pltpu.VMEM((D // 2 + 8, F), u32),
        pltpu.VMEM((F // 2 + 8, D), u32),
        pltpu.SemaphoreType.DMA((NSEM,)),
        pltpu.SMEM((1,), jnp.int32),
        pltpu.VMEM((2, S, 128), f32),
    ] + [pltpu.VMEM((H // 8, RING, DH), f32)] * 8
    out = pl.pallas_call(
        _kernel,
        out_shape=jax.ShapeDtypeStruct((S, D), A_x.dtype),
        in_specs=[hbm, vmem] + [hbm] * 8,
        out_specs=hbm,
        scratch_shapes=scratch,
        compiler_params=pltpu.CompilerParams(vmem_limit_bytes=255 * 512 * 1024),
    )(A_x.reshape(S, D), A_mem0.reshape(MEM, D),
      A_Wq, A_Wk, A_Wv,
      A_Wo.reshape(H * DH, D), B_w1, B_w2, B_w3, B_w4)
    return out.reshape(A_x.shape)
```
